```python
import jax
import jax.numpy as jnp

def _softmax(x, axis=-1):
    return jax.nn.softmax(x, axis=axis)
def _gelu(x):
    return jax.nn.gelu(x, approximate=True)
def _silu(x):
    return jax.nn.silu(x)
def _sigmoid(x):
    return jax.nn.sigmoid(x)
def _layernorm(x, axis=-1, eps=1e-5):
    m = jnp.mean(x, axis=axis, keepdims=True)
    v = jnp.var(x, axis=axis, keepdims=True)
    return (x - m) / jnp.sqrt(v + eps)
def _scatter_add(tgt, idx, src, axis=0):
    return tgt.at[idx].add(src)
def _segment_sum(src, seg, n):
    return jax.ops.segment_sum(src, seg, n)
class _Rng:
    def __init__(self, key):
        self._k = key
    def _next(self):
        self._k, sub = jax.random.split(self._k)
        return sub
    def normal(self, shape):
        return jax.random.normal(self._next(), shape, dtype=jnp.bfloat16)
    def randint(self, lo, hi, shape):
        return jax.random.randint(self._next(), shape, lo, hi, dtype=jnp.int32)
    def uniform(self, shape, lo=0.0, hi=1.0):
        return jax.random.uniform(self._next(), shape, jnp.bfloat16, lo, hi)
    def permutation(self, n):
        return jax.random.permutation(self._next(), n)


kernel_name = 'recurrent_scan__compressed_kv_cla__dense_activation_gelu__decode'

def setup_inputs():
    _rng = _Rng(jax.random.key(int.from_bytes(__import__("os").urandom(4), "little")))
    _w = (lambda a: (lambda t: t.astype(jnp.bfloat16) if jnp.issubdtype(t.dtype, jnp.floating) else t)(jnp.asarray(a)))
    def _A_setup():
        B, H, Sq, Sk, D, M = 2, 32, 1, 16384, 128, 512
        Dc = 4 * D
        return {
            "x": _w((lambda *s: _rng.normal(s) * 0.05)(B, Sq, M)),
            "c_kv": _w((lambda *s: _rng.normal(s) * 0.05)(B, Sk, Dc)),
            "w_q": _w((lambda *s: _rng.normal(s) * 0.05)(M, H, D) * (M ** -0.5)),
            "w_uk": _w((lambda *s: _rng.normal(s) * 0.05)(Dc, H, D) * (Dc ** -0.5)),
            "w_uv": _w((lambda *s: _rng.normal(s) * 0.05)(Dc, H, D) * (Dc ** -0.5)),
            "w_o": _w((lambda *s: _rng.normal(s) * 0.05)(H, D, M) * ((H * D) ** -0.5)),
        }
    _A_in = _A_setup()

    def _B_setup():
        B, S, D, F = 2, 1, 512, 1792
        return {
            "x": _w((lambda *s: _rng.normal(s) * 0.05)(B, S, D)),
            "w1": _w((lambda *s: _rng.normal(s) * 0.05)(D, F) * (D ** -0.5)),
            "b1": _w((lambda *s: _rng.normal(s) * 0.05)(F) * 0.01),
            "w2": _w((lambda *s: _rng.normal(s) * 0.05)(F, D) * (F ** -0.5)),
            "b2": _w((lambda *s: _rng.normal(s) * 0.05)(D) * 0.01),
        }
    _B_in = _B_setup()

    return {
        "A_x": _A_in["x"],
        "A_c_kv": _A_in["c_kv"],
        "A_w_q": _A_in["w_q"],
        "A_w_uk": _A_in["w_uk"],
        "A_w_uv": _A_in["w_uv"],
        "A_w_o": _A_in["w_o"],
        "B_x": _B_in["x"],
        "B_w1": _B_in["w1"],
        "B_b1": _B_in["b1"],
        "B_w2": _B_in["w2"],
        "B_b2": _B_in["b2"],
    }

def reference(A_x, A_c_kv, A_w_q, A_w_uk, A_w_uv, A_w_o, B_x, B_w1, B_b1, B_w2, B_b2):
    def _A_ref(x, c_kv, w_q, w_uk, w_uv, w_o):
        B, Sq, M = x.shape[0], x.shape[1], x.shape[2]
        Sk = c_kv.shape[1]
        H, D = w_q.shape[1], w_q.shape[2]
        q = jnp.einsum("bqm,mhd->bhqd", x, w_q)
        k = jnp.einsum("bkc,chd->bhkd", c_kv, w_uk)
        v = jnp.einsum("bkc,chd->bhkd", c_kv, w_uv)
        scores = jnp.einsum("bhqd,bhkd->bhqk", q, k) * (D ** -0.5)
        off = Sk - Sq
        qi = jnp.arange(Sq)[:, None]
        kj = jnp.arange(Sk)[None, :]
        cmask = kj <= (qi + off)
        scores = jnp.where(cmask[None, None], scores, -1e9)
        p = _softmax(scores, axis=-1)
        ctx = jnp.einsum("bhqk,bhkd->bhqd", p, v)
        return jnp.einsum("bhqd,hdm->bqm", ctx, w_o)

    def _B_ref(x, w1, b1, w2, b2):
        h = jnp.einsum("bsd,df->bsf", x, w1) + b1
        h = _gelu(h)
        return jnp.einsum("bsf,fd->bsd", h, w2) + b2

    x = A_x
    xn = _layernorm(x, axis=-1)
    s = _A_ref(xn, A_c_kv, A_w_q, A_w_uk, A_w_uv, A_w_o)
    g = _silu(_B_ref(xn, B_w1, B_b1, B_w2, B_b2))
    return x + s * g
```

```python
import jax
import jax.numpy as jnp
from jax import lax
import jax.experimental.pallas as pl
import jax.experimental.pallas.tpu as pltpu

F32 = jnp.float32
BF16 = jnp.bfloat16
B, H, SK, D, M, DC, F = 2, 32, 16384, 128, 512, 512, 1792
LOG2E = 1.4426950408889634
NT = (((1,), (1,)), ((), ()))


def make_kernel(S=1600, P=128, INIT=3, K=5, CS=32, BJ=4, tail=(256, 128, 128), ffn_at=4, xn_smem=False, SU=4, IU=1, flags=None, prof=False):
    def mark(name):
        if prof:
            with jax.named_scope(name):
                pl.delay(1)
    NPC = -(-S // P)
    CN = SK // (CS * 32)
    NQ = 8
    QJ = B * CS // NQ
    NO = 8 - sum(tail) // 512
    LAST = 10

    def kernel(x_hbm, ckv_hbm, wq_hbm, wuk_hbm, wuv_hbm, wo_hbm, w1_hbm, b1_hbm, w2_hbm, b2_hbm,
               o_ref,
               x_buf, b1_buf, b2_buf, c_buf, wq_buf, wuk_buf, wuv_buf, wo_buf, w1_buf, w2_buf, ring,
               xn_vmem, xs, t8, qa_ref, acc_ref, m_ref, l_ref, a_buf, ctx_ref, sems, ring_sems, sem_small):
        def copy(src, dst, sem):
            return pltpu.make_async_copy(src, dst, sem)

        def start_weight(hbm, buf, sem):
            @pl.loop(0, 16, unroll=IU)
            def _(j):
                copy(hbm.at[:, j], buf.at[:, j], sem).start(priority=1)

        def wait_all(buf, sem):
            copy(buf, buf, sem).wait()

        def quad(q):
            return q // (NQ // B), (q % (NQ // B)) * QJ

        def start_quad(q):
            b, j0 = quad(q)
            @pl.loop(0, QJ, unroll=IU)
            def _(j):
                copy(ckv_hbm.at[b, :, j0 + j], c_buf.at[b, j0 + j], sems.at[q % 2]).start(priority=1)

        def piece(p):
            if isinstance(p, int):
                n = min(P, S - p * P)
                return pl.ds(p * P, n), ring.at[p % K, pl.ds(0, n)], ring_sems.at[p % K]
            return pl.ds(pl.multiple_of(p * P, P), P), ring.at[p % K], ring_sems.at[p % K]

        def to_smem(p):
            rows, slot, sem = piece(p)
            return copy(w2_hbm.at[rows], slot, sem)

        def to_vmem(p):
            rows, slot, sem = piece(p)
            return copy(slot, w2_buf.at[rows], sem)

        def service(k):
            to_smem(k).wait()
            to_vmem(k).start()
            p = k + INIT
            if isinstance(k, int):
                if p >= K:
                    to_vmem(p - K).wait()
                to_smem(p).start()
            else:
                pl.when((p >= K) & (p < NPC))(lambda: to_vmem(p - K).wait())
                pl.when(p < S // P)(lambda: to_smem(p).start())
                if S % P:
                    pl.when(p == NPC - 1)(lambda: to_smem(NPC - 1).start())

        x_copy = copy(x_hbm, x_buf, sem_small.at[0])
        b1_copy = copy(b1_hbm, b1_buf, sem_small.at[1])
        b2_copy = copy(b2_hbm, b2_buf, sem_small.at[1])
        start_weight(wq_hbm, wq_buf, sems.at[0])
        for p in range(INIT):
            to_smem(p).start()
        x_copy.start(priority=1)
        start_weight(wuk_hbm, wuk_buf, sems.at[1])
        b1_copy.start(priority=1)
        b2_copy.start(priority=1)

        mark('issued')
        wait_all(wq_buf, sems.at[0])
        mark('wq')
        service(0)
        start_quad(0)
        x_copy.wait()
        x = x_buf[...].astype(F32)
        xc = x - jnp.mean(x, axis=-1, keepdims=True)
        var = jnp.mean(xc * xc, axis=-1, keepdims=True)
        xn = (xc * lax.rsqrt(var + 1e-5)).astype(BF16)
        if xn_smem:
            xn_vmem[...] = xn.astype(F32)
            c = copy(xn_vmem, xs, sem_small.at[0])
            c.start()
            c.wait()
        else:
            xp = jnp.concatenate([xn.astype(F32), jnp.zeros((128 - B, M), F32)], axis=0)
            for j in range(M // 128):
                xt = xp[:, j * 128:(j + 1) * 128].T
                for b in range(B):
                    xn_vmem[b, j * 128:(j + 1) * 128, :] = jnp.broadcast_to(xt[:, b:b + 1], (128, 128))

        def q_body(t, carry):
            q0, q1 = carry
            for u in range(8):
                m = t * 8 + u
                w = wq_buf[t // 8, (t % 8) * 2 + u // 4, u % 4].astype(F32)
                if xn_smem:
                    q0 = q0 + xs[0, m] * w
                    q1 = q1 + xs[1, m] * w
                else:
                    q0 = q0 + xn_vmem[0, pl.ds(m, 1), :] * w
                    q1 = q1 + xn_vmem[1, pl.ds(m, 1), :] * w
            return q0, q1

        q01 = lax.fori_loop(0, M // 8, q_body, (jnp.zeros((H, D), F32), jnp.zeros((H, D), F32)))
        q = jnp.concatenate([q01[0], q01[1], jnp.zeros((128 - B * H, D), F32)], axis=0).astype(BF16)

        mark('q_done')
        wait_all(wuk_buf, sems.at[1])
        mark('wuk')
        service(1)
        start_quad(1)
        group = (lax.broadcasted_iota(jnp.int32, (16, 8, 128), 2) % H) // 8

        def qa_body(s, _):
            u = wuk_buf[s // 4, pl.ds((s % 4) * 4, 4)].reshape(16 * H, D)
            r = lax.dot_general(u, q, NT, preferred_element_type=F32).reshape(16, 4, 8, 128)
            v = jnp.where(group == 0, r[:, 0],
                          jnp.where(group == 1, r[:, 1], jnp.where(group == 2, r[:, 2], r[:, 3])))
            t8[pl.ds(pl.multiple_of(s * 128, 128), 128), :] = v.reshape(128, 128)

        lax.fori_loop(0, DC // 16, qa_body, None, unroll=2)
        sub = lax.broadcasted_iota(jnp.int32, (128, 128), 1) % 8
        for j in range(DC // 128):
            t = t8[pl.ds(j * 1024, 128, stride=8), :]
            for s in range(1, 8):
                t = jnp.where(sub == s, t8[pl.ds(j * 1024 + s, 128, stride=8), :], t)
            qa_ref[:, j * 128:(j + 1) * 128] = (t.T[:B * H] * (D ** -0.5 * LOG2E)).astype(BF16)

        m_ref[...] = jnp.full((B * H, 128), -jnp.inf, F32)
        l_ref[...] = jnp.zeros((B * H, 128), F32)
        acc_ref[...] = jnp.zeros((B * H, DC), F32)
        rest = pl.ds(S, F - S)
        ffn_copies = [copy(w1_hbm, w1_buf, sems.at[1]), copy(w2_hbm.at[rest], w2_buf.at[rest], sems.at[1])]

        def chunk(qi, _):
            b, j0 = quad(qi)
            mark('c_ready')
            wait_all(c_buf.at[b, pl.ds(j0, QJ)], sems.at[qi % 2])
            mark('c_arr')
            service(qi + 2)
            mark('c_srv')
            pl.when(qi + 2 < NQ)(lambda: start_quad(qi + 2))
            pl.when(qi == NQ - 2)(lambda: start_weight(wuv_hbm, wuv_buf, sems.at[0]))

            @pl.when(qi == NQ - 1)
            def _():
                for c in ffn_copies:
                    c.start(priority=1)

            hrows = pl.ds(pl.multiple_of(b * H, H), H)

            def block(jj, _):
                c = c_buf[b, pl.ds(j0 + jj * BJ, BJ)].reshape(BJ * CN * 32, DC)
                sc = lax.dot_general(qa_ref[hrows, :], c, NT, preferred_element_type=F32)
                m_prev = m_ref[hrows, :]
                m_new = jnp.maximum(m_prev, jnp.max(sc, axis=1, keepdims=True))
                p = jnp.exp2(sc - m_new[:, :1])
                alpha = jnp.exp2(m_prev - m_new)
                l_ref[hrows, :] = alpha * l_ref[hrows, :] + jnp.sum(p, axis=1, keepdims=True)
                m_ref[hrows, :] = m_new
                pv = jnp.dot(p.astype(BF16), c, preferred_element_type=F32)
                acc_ref[hrows, :] = acc_ref[hrows, :] * alpha[:, :1] + pv

            lax.fori_loop(0, QJ // BJ, block, None)

        lax.fori_loop(0, NQ, chunk, None)

        mark('att_done')
        pc = (acc_ref[...] / l_ref[...][:, :1]).astype(BF16)
        pcs = jnp.concatenate([pc[:, j * 128:(j + 1) * 128] for j in range(DC // 128)], axis=0)
        lane = lax.broadcasted_iota(jnp.int32, (4 * B * H, 128), 1)
        diag = (lane % H) == lax.broadcasted_iota(jnp.int32, (4 * B * H, 128), 0) % H
        src = lax.broadcasted_iota(jnp.int32, (128, 128), 0) - lax.broadcasted_iota(jnp.int32, (128, 128), 1) // H

        def spread(t, _):
            rep = jnp.dot(pcs, jnp.where(src == 4 * t, 1.0, 0.0).astype(BF16), preferred_element_type=F32)
            a_buf[:, t] = jnp.where(diag, rep, 0.0).astype(BF16).reshape(4, B * H, 128)

        lax.fori_loop(0, 32, spread, None, unroll=SU)
        mark('lhs_done')
        wait_all(wuv_buf, sems.at[0])
        mark('wuv')
        for p in range(LAST, NPC):
            to_smem(p).wait()
            to_vmem(p).start()
        @pl.loop(0, 16, unroll=IU)
        def _(j):
            copy(wo_hbm.at[pl.ds(0, NO), j], wo_buf.at[pl.ds(0, NO), j], sems.at[2 + j // 4]).start(priority=1)
        tails = []
        o = 0
        for t, n in enumerate(tail):
            i, j = NO + o // 512, (o % 512) // 32
            idx = (i, pl.ds(j, n // 32))
            tails.append((o, n, idx, copy(wo_hbm.at[idx], wo_buf.at[idx], sems.at[6 + t])))
            tails[-1][-1].start(priority=1)
            o += n

        def ctx_body(j, ctx):
            lhs = jnp.concatenate([a_buf[j, t] for t in range(32)], axis=1)
            v2 = wuv_buf[pl.ds(2 * j, 2)].reshape(128 * H, D)
            return ctx + jnp.dot(lhs, v2, preferred_element_type=F32)

        ctx_ref[...] = lax.fori_loop(0, DC // 128, ctx_body, jnp.zeros((B * H, D), F32))
        mark('ctx_done')

        def ctx_head(h):
            return ctx_ref[pl.ds(h, B, stride=H), :].astype(BF16)

        b1_copy.wait()
        b2_copy.wait()
        for c in ffn_copies:
            c.wait()
        h = jnp.dot(xn, w1_buf[...], preferred_element_type=F32) + b1_buf[...].astype(F32).reshape(1, F)
        h = jax.nn.gelu(h, approximate=True).astype(BF16)
        early = LAST * P
        for p in range(NPC - K, LAST):
            to_vmem(p).wait()
        gg = b2_buf[...].astype(F32).reshape(1, M)
        gg = gg + jnp.dot(h[:, :early], w2_buf[pl.ds(0, early), :], preferred_element_type=F32)

        mark('ffn1_done')
        s = jnp.zeros((B, M), F32)
        steps = []
        for g in range(4):
            def step(s, g=g):
                v = wo_buf.at[pl.ds(0, NO), pl.ds(4 * g, 4)]
                mark('wo_ready')
                wait_all(v, sems.at[2 + g])
                mark('wo_arr')
                lhs = jnp.concatenate([ctx_head(4 * i + g) for i in range(NO)], axis=1)
                return s + jnp.dot(lhs, wo_buf[pl.ds(0, NO), pl.ds(4 * g, 4)].reshape(NO * D, M), preferred_element_type=F32)
            steps.append(step)
        lhs_tail = jnp.concatenate([ctx_head(hh) for hh in range(4 * NO, H)], axis=1)
        for o, n, idx, c in tails:
            def step(s, o=o, n=n, idx=idx, c=c):
                mark('t_ready')
                c.wait()
                mark('t_arr')
                return s + jnp.dot(lhs_tail[:, o:o + n], wo_buf[idx].reshape(n, M), preferred_element_type=F32)
            steps.append(step)
        for i, step in enumerate(steps[:-1]):
            if i == ffn_at:
                for p in range(LAST, NPC):
                    to_vmem(p).wait()
                mark('ring_done')
                gg = gg + jnp.dot(h[:, early:], w2_buf[pl.ds(early, F - early), :], preferred_element_type=F32)
                gate = gg * jax.nn.sigmoid(gg)
            s = step(s)
        base = x + s * gate
        o_ref[...] = (base + steps[-1](jnp.zeros((B, M), F32)) * gate).astype(BF16)

    def fn(A_x, A_c_kv, A_w_q, A_w_uk, A_w_uv, A_w_o, B_x, B_w1, B_b1, B_w2, B_b2):
        del B_x
        W = (8, 16, 4, H, D)
        WO = (8, 16, 32, M)
        out = pl.pallas_call(
            kernel,
            out_shape=jax.ShapeDtypeStruct((B, M), BF16),
            in_specs=[pl.BlockSpec(memory_space=pltpu.HBM)] * 10,
            out_specs=pl.BlockSpec(memory_space=pltpu.VMEM),
            scratch_shapes=[
                pltpu.VMEM((B, M), BF16), pltpu.VMEM((F,), BF16), pltpu.VMEM((M,), BF16),
                pltpu.VMEM((B, CS, CN, 32, DC), BF16),
                pltpu.VMEM(W, BF16), pltpu.VMEM(W, BF16), pltpu.VMEM(W, BF16),
                pltpu.VMEM(WO, BF16), pltpu.VMEM((M, F), BF16), pltpu.VMEM((F, M), BF16),
                pltpu.SMEM((K, P, M), BF16),
                pltpu.VMEM((B, M) if xn_smem else (B, M, 128), F32), pltpu.SMEM((B, M), F32),
                pltpu.VMEM((DC * 8 + 8, 128), F32),
                pltpu.VMEM((B * H, DC), BF16), pltpu.VMEM((B * H, DC), F32),
                pltpu.VMEM((B * H, 128), F32), pltpu.VMEM((B * H, 128), F32),
                pltpu.VMEM((4, 32, B * H, 128), BF16), pltpu.VMEM((B * H, D), F32),
                pltpu.SemaphoreType.DMA((6 + len(tail),)), pltpu.SemaphoreType.DMA((K,)), pltpu.SemaphoreType.DMA((2,)),
            ],
            compiler_params=pltpu.CompilerParams(vmem_limit_bytes=100 * 1024 * 1024, disable_bounds_checks=True,
                                                 disable_semaphore_checks=True, flags=flags),
        )(A_x.reshape(B, M), A_c_kv.reshape(B, CN, CS, 32, DC), A_w_q.reshape(W), A_w_uk.reshape(W), A_w_uv.reshape(W),
          A_w_o.reshape(WO), B_w1, B_b1, B_w2, B_b2)
        return out.reshape(B, 1, M)
    return fn


_impl = make_kernel(**dict(S=1568,ffn_at=3))


@jax.jit
def pallas_recurrent_scan__compressed_kv_cla__dense_activation_gelu__decode_kernel(
    A_x: jax.Array,
    A_c_kv: jax.Array,
    A_w_q: jax.Array,
    A_w_uk: jax.Array,
    A_w_uv: jax.Array,
    A_w_o: jax.Array,
    B_x: jax.Array,
    B_w1: jax.Array,
    B_b1: jax.Array,
    B_w2: jax.Array,
    B_b2: jax.Array,
):
    return _impl(A_x, A_c_kv, A_w_q, A_w_uk, A_w_uv, A_w_o, B_x, B_w1, B_b1, B_w2, B_b2)
```

```python
import jax
import jax.numpy as jnp
from jax import lax
import jax.experimental.pallas as pl
import jax.experimental.pallas.tpu as pltpu

F32 = jnp.float32
BF16 = jnp.bfloat16
B, H, SK, D, M, DC, F = 2, 32, 16384, 128, 512, 512, 1792
LOG2E = 1.4426950408889634
NT = (((1,), (1,)), ((), ()))


def make_kernel(S=1600, P=128, INIT=3, K=5, CS=32, BJ=4, wo=(8, 8, 8, 4, 2, 1), vpu=(), mxu_last=128, ffn_at=(2, 3, 4), es=True, xn_smem=False, SU=4, IU=1, flags=None, prof=False):
    def mark(name):
        if prof:
            with jax.named_scope(name):
                pl.delay(1)
    NPC = -(-S // P)
    CN = SK // (CS * 32)
    NQ = 8
    QJ = B * CS // NQ
    WO = [n * D for n in wo] + ([mxu_last] if mxu_last else [])
    assert sum(WO) + sum(vpu) == H * D
    RV = sum(vpu)
    LAST = 10

    def kernel(x_hbm, ckv_hbm, wq_hbm, wuk_hbm, wuv_hbm, wo_hbm, w1_hbm, b1_hbm, w2_hbm, b2_hbm,
               o_ref,
               x_buf, b1_buf, b2_buf, c_buf, wq_buf, wuk_buf, wuv_buf, wo_buf, w1_buf, w2_buf, ring,
               xn_vmem, xs, t8, qa_ref, acc_ref, m_ref, l_ref, a_buf, ctx_ref, cb_ref, sems, ring_sems, sem_small):
        def copy(src, dst, sem):
            return pltpu.make_async_copy(src, dst, sem)

        def start_weight(hbm, buf, sem, first=0):
            @pl.loop(first, 16, unroll=IU)
            def _(j):
                copy(hbm.at[:, j], buf.at[:, j], sem).start(priority=1)

        def wait_all(buf, sem):
            copy(buf, buf, sem).wait()

        def quad(q):
            return q // (NQ // B), (q % (NQ // B)) * QJ

        def start_quad(q):
            b, j0 = quad(q)
            @pl.loop(0, QJ, unroll=IU)
            def _(j):
                copy(ckv_hbm.at[b, :, j0 + j], c_buf.at[b, j0 + j], sems.at[q % 2]).start(priority=1)

        def piece(p):
            if isinstance(p, int):
                n = min(P, S - p * P)
                return pl.ds(p * P, n), ring.at[p % K, pl.ds(0, n)], ring_sems.at[p % K]
            return pl.ds(pl.multiple_of(p * P, P), P), ring.at[p % K], ring_sems.at[p % K]

        def to_smem(p):
            rows, slot, sem = piece(p)
            return copy(w2_hbm.at[rows], slot, sem)

        def to_vmem(p):
            rows, slot, sem = piece(p)
            return copy(slot, w2_buf.at[rows], sem)

        def service(k):
            if not (es and isinstance(k, int) and k == 0):
                to_smem(k).wait()
                to_vmem(k).start()
            p = k + INIT
            if isinstance(k, int):
                if p >= K:
                    to_vmem(p - K).wait()
                to_smem(p).start()
            else:
                pl.when((p >= K) & (p < NPC))(lambda: to_vmem(p - K).wait())
                pl.when(p < S // P)(lambda: to_smem(p).start())
                if S % P:
                    pl.when(p == NPC - 1)(lambda: to_smem(NPC - 1).start())

        x_copy = copy(x_hbm, x_buf, sem_small.at[0])
        b1_copy = copy(b1_hbm, b1_buf, sem_small.at[1])
        b2_copy = copy(b2_hbm, b2_buf, sem_small.at[1])
        copy(wq_hbm.at[:, 0], wq_buf.at[:, 0], sems.at[0]).start(priority=1)
        for p in range(INIT):
            to_smem(p).start()
        start_weight(wq_hbm, wq_buf, sems.at[0], 1)
        x_copy.start(priority=1)
        start_weight(wuk_hbm, wuk_buf, sems.at[1])
        b1_copy.start(priority=1)
        b2_copy.start(priority=1)

        mark('issued')
        if es:
            to_smem(0).wait()
            to_vmem(0).start()
        wait_all(wq_buf, sems.at[0])
        mark('wq')
        service(0)
        start_quad(0)
        x_copy.wait()
        x = x_buf[...].astype(F32)
        xc = x - jnp.mean(x, axis=-1, keepdims=True)
        var = jnp.mean(xc * xc, axis=-1, keepdims=True)
        xn = (xc * lax.rsqrt(var + 1e-5)).astype(BF16)
        if xn_smem:
            xn_vmem[...] = xn.astype(F32)
            c = copy(xn_vmem, xs, sem_small.at[0])
            c.start()
            c.wait()
        else:
            xp = jnp.concatenate([xn.astype(F32), jnp.zeros((128 - B, M), F32)], axis=0)
            for j in range(M // 128):
                xt = xp[:, j * 128:(j + 1) * 128].T
                for b in range(B):
                    xn_vmem[b, j * 128:(j + 1) * 128, :] = jnp.broadcast_to(xt[:, b:b + 1], (128, 128))

        def q_body(t, carry):
            q0, q1 = carry
            for u in range(8):
                m = t * 8 + u
                w = wq_buf[t // 8, (t % 8) * 2 + u // 4, u % 4].astype(F32)
                if xn_smem:
                    q0 = q0 + xs[0, m] * w
                    q1 = q1 + xs[1, m] * w
                else:
                    q0 = q0 + xn_vmem[0, pl.ds(m, 1), :] * w
                    q1 = q1 + xn_vmem[1, pl.ds(m, 1), :] * w
            return q0, q1

        q01 = lax.fori_loop(0, M // 8, q_body, (jnp.zeros((H, D), F32), jnp.zeros((H, D), F32)))
        q = jnp.concatenate([q01[0], q01[1], jnp.zeros((128 - B * H, D), F32)], axis=0).astype(BF16)

        mark('q_done')
        wait_all(wuk_buf, sems.at[1])
        mark('wuk')
        service(1)
        start_quad(1)
        group = (lax.broadcasted_iota(jnp.int32, (16, 8, 128), 2) % H) // 8

        def qa_body(s, _):
            u = wuk_buf[s // 4, pl.ds((s % 4) * 4, 4)].reshape(16 * H, D)
            r = lax.dot_general(u, q, NT, preferred_element_type=F32).reshape(16, 4, 8, 128)
            v = jnp.where(group == 0, r[:, 0],
                          jnp.where(group == 1, r[:, 1], jnp.where(group == 2, r[:, 2], r[:, 3])))
            t8[pl.ds(pl.multiple_of(s * 128, 128), 128), :] = v.reshape(128, 128)

        lax.fori_loop(0, DC // 16, qa_body, None, unroll=2)
        sub = lax.broadcasted_iota(jnp.int32, (128, 128), 1) % 8
        for j in range(DC // 128):
            t = t8[pl.ds(j * 1024, 128, stride=8), :]
            for s in range(1, 8):
                t = jnp.where(sub == s, t8[pl.ds(j * 1024 + s, 128, stride=8), :], t)
            qa_ref[:, j * 128:(j + 1) * 128] = (t.T[:B * H] * (D ** -0.5 * LOG2E)).astype(BF16)

        m_ref[...] = jnp.full((B * H, 128), -jnp.inf, F32)
        l_ref[...] = jnp.zeros((B * H, 128), F32)
        acc_ref[...] = jnp.zeros((B * H, DC), F32)
        rest = pl.ds(S, F - S)
        ffn_copies = [copy(w1_hbm, w1_buf, sems.at[1]), copy(w2_hbm.at[rest], w2_buf.at[rest], sems.at[1])]

        def chunk(qi, _):
            b, j0 = quad(qi)
            mark('c_ready')
            wait_all(c_buf.at[b, pl.ds(j0, QJ)], sems.at[qi % 2])
            mark('c_arr')
            service(qi + 2)
            mark('c_srv')
            pl.when(qi + 2 < NQ)(lambda: start_quad(qi + 2))
            pl.when(qi == NQ - 2)(lambda: start_weight(wuv_hbm, wuv_buf, sems.at[0]))

            @pl.when(qi == NQ - 1)
            def _():
                for c in ffn_copies:
                    c.start(priority=1)

            hrows = pl.ds(pl.multiple_of(b * H, H), H)

            def block(jj, _):
                c = c_buf[b, pl.ds(j0 + jj * BJ, BJ)].reshape(BJ * CN * 32, DC)
                sc = lax.dot_general(qa_ref[hrows, :], c, NT, preferred_element_type=F32)
                m_prev = m_ref[hrows, :]
                m_new = jnp.maximum(m_prev, jnp.max(sc, axis=1, keepdims=True))
                p = jnp.exp2(sc - m_new[:, :1])
                alpha = jnp.exp2(m_prev - m_new)
                l_ref[hrows, :] = alpha * l_ref[hrows, :] + jnp.sum(p, axis=1, keepdims=True)
                m_ref[hrows, :] = m_new
                pv = jnp.dot(p.astype(BF16), c, preferred_element_type=F32)
                acc_ref[hrows, :] = acc_ref[hrows, :] * alpha[:, :1] + pv

            lax.fori_loop(0, QJ // BJ, block, None)

        lax.fori_loop(0, NQ, chunk, None)

        mark('att_done')
        pc = (acc_ref[...] / l_ref[...][:, :1]).astype(BF16)
        pcs = jnp.concatenate([pc[:, j * 128:(j + 1) * 128] for j in range(DC // 128)], axis=0)
        lane = lax.broadcasted_iota(jnp.int32, (4 * B * H, 128), 1)
        diag = (lane % H) == lax.broadcasted_iota(jnp.int32, (4 * B * H, 128), 0) % H
        src = lax.broadcasted_iota(jnp.int32, (128, 128), 0) - lax.broadcasted_iota(jnp.int32, (128, 128), 1) // H

        def spread(t, _):
            rep = jnp.dot(pcs, jnp.where(src == 4 * t, 1.0, 0.0).astype(BF16), preferred_element_type=F32)
            a_buf[:, t] = jnp.where(diag, rep, 0.0).astype(BF16).reshape(4, B * H, 128)

        lax.fori_loop(0, 32, spread, None, unroll=SU)
        mark('lhs_done')
        wait_all(wuv_buf, sems.at[0])
        mark('wuv')
        for p in range(LAST, NPC):
            to_smem(p).wait()
            to_vmem(p).start()
        pieces = []
        o = 0
        for t, n in enumerate(WO + list(vpu)):
            pieces.append((o, n, copy(wo_hbm.at[pl.ds(o, n)], wo_buf.at[pl.ds(o, n)], sems.at[2 + t])))
            pieces[-1][-1].start(priority=1)
            o += n

        def ctx_body(j, ctx):
            lhs = jnp.concatenate([a_buf[j, t] for t in range(32)], axis=1)
            v2 = wuv_buf[pl.ds(2 * j, 2)].reshape(128 * H, D)
            return ctx + jnp.dot(lhs, v2, preferred_element_type=F32)

        ctx_ref[...] = lax.fori_loop(0, DC // 128, ctx_body, jnp.zeros((B * H, D), F32))
        mark('ctx_done')

        def ctx_rows(o, n):
            hs = range(o // D, -(-(o + n) // D))
            v = jnp.concatenate([ctx_ref[pl.ds(h, B, stride=H), :] for h in hs], axis=1)
            v = jnp.concatenate([v, jnp.zeros((8 - B, v.shape[1]), F32)], axis=0)
            return v[:, o % D:o % D + n].astype(BF16)

        for t in range(-(-RV // D)):
            hh = H - 1 - t
            ct = jnp.concatenate([ctx_ref[pl.ds(hh, B, stride=H), :], jnp.zeros((128 - B, D), F32)], axis=0).T
            for b in range(B):
                cb_ref[b, pl.ds(cb_ref.shape[1] - (t + 1) * D, D), :] = jnp.broadcast_to(ct[:, b:b + 1], (D, 128))

        b1_copy.wait()
        b2_copy.wait()
        for c in ffn_copies:
            c.wait()
        xn8 = jnp.concatenate([xn.astype(F32), jnp.zeros((8 - B, M), F32)], axis=0).astype(BF16)
        h = jnp.dot(xn8, w1_buf[...], preferred_element_type=F32) + b1_buf[...].astype(F32).reshape(1, F)
        h = jax.nn.gelu(h, approximate=True).astype(BF16)
        early = LAST * P
        for p in range(NPC - K, LAST):
            to_vmem(p).wait()

        def w2_dot(o, e):
            return jnp.dot(h[:, o:e], w2_buf[pl.ds(o, e - o), :], preferred_element_type=F32)

        gg = b2_buf[...].astype(F32).reshape(1, M) + w2_dot(0, early)
        if NPC * P < F:
            gg = gg + w2_dot(NPC * P, F)
        mark('ffn1_done')

        x8 = jnp.concatenate([x, jnp.zeros((8 - B, M), F32)], axis=0)
        s = jnp.zeros((8, M), F32)
        acc = [None] * B
        for i, (o, n, c) in enumerate(pieces):
            for p, at in zip(range(LAST, NPC), ffn_at):
                if at == i:
                    to_vmem(p).wait()
                    mark('ring')
                    gg = gg + w2_dot(p * P, (p + 1) * P)
                    if p == NPC - 1:
                        gate = gg * jax.nn.sigmoid(gg)
            if i < len(WO):
                lhs = ctx_rows(o, n)
                if i == len(pieces) - 1:
                    base = x8 + s * gate
                mark('wo_ready')
                c.wait()
                mark('wo_arr')
                r = jnp.dot(lhs, wo_buf[pl.ds(o, n), :], preferred_element_type=F32)
                if i == len(pieces) - 1:
                    o_ref[...] = (base + r * gate).astype(BF16)[:B]
                s = s + r
            else:
                if i == len(pieces) - 1:
                    base = x8 + s * gate
                mark('v_ready')
                c.wait()
                mark('v_arr')
                for r0 in range(o, o + n, 8):
                    w = wo_buf[pl.ds(r0, 8), :].astype(F32)
                    for b in range(B):
                        a = cb_ref[b, pl.ds(r0 - H * D + cb_ref.shape[1], 8), :]
                        t = w * jnp.concatenate([a] * (M // 128), axis=1)
                        acc[b] = t if acc[b] is None else acc[b] + t
        if vpu:
            row = lax.broadcasted_iota(jnp.int32, (8, M), 0)
            r = [jnp.sum(acc[b], axis=0, keepdims=True) for b in range(B)]
            r = jnp.where(row == 0, r[0], r[1])
            o_ref[...] = (base + r * gate).astype(BF16)[:B]

    def fn(A_x, A_c_kv, A_w_q, A_w_uk, A_w_uv, A_w_o, B_x, B_w1, B_b1, B_w2, B_b2):
        del B_x
        W = (8, 16, 4, H, D)
        out = pl.pallas_call(
            kernel,
            out_shape=jax.ShapeDtypeStruct((B, M), BF16),
            in_specs=[pl.BlockSpec(memory_space=pltpu.HBM)] * 10,
            out_specs=pl.BlockSpec(memory_space=pltpu.VMEM),
            scratch_shapes=[
                pltpu.VMEM((B, M), BF16), pltpu.VMEM((F,), BF16), pltpu.VMEM((M,), BF16),
                pltpu.VMEM((B, CS, CN, 32, DC), BF16),
                pltpu.VMEM(W, BF16), pltpu.VMEM(W, BF16), pltpu.VMEM(W, BF16),
                pltpu.VMEM((H * D, M), BF16), pltpu.VMEM((M, F), BF16), pltpu.VMEM((F, M), BF16),
                pltpu.SMEM((K, P, M), BF16),
                pltpu.VMEM((B, M) if xn_smem else (B, M, 128), F32), pltpu.SMEM((B, M), F32),
                pltpu.VMEM((DC * 8 + 8, 128), F32),
                pltpu.VMEM((B * H, DC), BF16), pltpu.VMEM((B * H, DC), F32),
                pltpu.VMEM((B * H, 128), F32), pltpu.VMEM((B * H, 128), F32),
                pltpu.VMEM((4, 32, B * H, 128), BF16), pltpu.VMEM((B * H, D), F32),
                pltpu.VMEM((B, max(1, -(-RV // D)) * D, 128), F32),
                pltpu.SemaphoreType.DMA((2 + len(WO) + len(vpu),)), pltpu.SemaphoreType.DMA((K,)), pltpu.SemaphoreType.DMA((2,)),
            ],
            compiler_params=pltpu.CompilerParams(vmem_limit_bytes=100 * 1024 * 1024, disable_bounds_checks=True,
                                                 disable_semaphore_checks=True, flags=flags),
        )(A_x.reshape(B, M), A_c_kv.reshape(B, CN, CS, 32, DC), A_w_q.reshape(W), A_w_uk.reshape(W), A_w_uv.reshape(W),
          A_w_o.reshape(H * D, M), B_w1, B_b1, B_w2, B_b2)
        return out.reshape(B, 1, M)
    return fn


_impl = make_kernel(**dict(mxu_last=0,wo=(8,8,8,4,2),vpu=(128,64,32,32),S=1608))


@jax.jit
def pallas_recurrent_scan__compressed_kv_cla__dense_activation_gelu__decode_kernel(
    A_x: jax.Array,
    A_c_kv: jax.Array,
    A_w_q: jax.Array,
    A_w_uk: jax.Array,
    A_w_uv: jax.Array,
    A_w_o: jax.Array,
    B_x: jax.Array,
    B_w1: jax.Array,
    B_b1: jax.Array,
    B_w2: jax.Array,
    B_b2: jax.Array,
):
    return _impl(A_x, A_c_kv, A_w_q, A_w_uk, A_w_uv, A_w_o, B_x, B_w1, B_b1, B_w2, B_b2)
```

```python
import jax
import jax.numpy as jnp
from jax import lax
import jax.experimental.pallas as pl
import jax.experimental.pallas.tpu as pltpu

F32 = jnp.float32
BF16 = jnp.bfloat16
B, H, SK, D, M, DC, F = 2, 32, 16384, 128, 512, 512, 1792
LOG2E = 1.4426950408889634
NT = (((1,), (1,)), ((), ()))


def _order(bits):
    return [sum(((c >> k) & 1) << b for k, b in enumerate(bits)) for c in range(1 << len(bits))]


def make_kernel(wb=(4, 5, 6, 3, 2), cb=(0, 5, 6, 7, 8), ob=(5, 6, 4, 0, 1), lead=27, vpu=(128, 64, 32, 32), tiny=8,
                first=32, QU=4, chunk=16, flags=None, prof=False, noatt=False):
    def mark(name):
        if prof:
            with jax.named_scope(name):
                pl.delay(1)

    AHEAD = 3
    NS = AHEAD + 1
    NCB = 32
    VH = (27, 31)
    assert sum(vpu) == len(VH) * D

    def kernel(x_hbm, ckv_hbm, wq_hbm, wuk_hbm, wuv_hbm, wo_hbm, w1_hbm, b1_hbm, w2_hbm, b2_hbm,
               o_ref,
               x_buf, b1_buf, b2_buf, c_buf, wq_buf, wuk_buf, wuv_buf, wo_buf, w1_buf, w2_buf,
               xb_ref, t8, qa_ref, acc_ref, m_ref, l_ref, a_buf, ctx_ref, cb_ref, sems, tsems, sem_small):
        def copy(src, dst, sem):
            return pltpu.make_async_copy(src, dst, sem)

        def wait_all(buf, sem):
            copy(buf, buf, sem).wait()

        def start_weight(hbm, buf, y, slot, bulk=0):
            for k, g in enumerate(_order(wb)):
                copy(hbm.at[g + y], buf.at[y, g // 32, (g % 32) // 4], sems.at[slot % NS]).start(priority=1 if k < bulk else k % 2)

        cfree = [b for b in range(10) if b not in cb]

        def start_ckv(i):
            base = sum(((i >> k) & 1) << b for k, b in enumerate(cfree))
            for k, g in enumerate(_order(cb)):
                copy(ckv_hbm.at[base + g], c_buf.at[i, k], sems.at[i % NS]).start(priority=k % 2)

        def rows(hbm, buf, o, n, s):
            return (hbm.at[pl.ds(o, n)], buf.at[pl.ds(o, n)], s)

        seq = []
        r6 = _order((5, 4, 3, 2, 1, 0))
        r2 = [g for g in r6 if g < F // 32]
        for k in range(64):
            if k < len(r2):
                seq.append((w2_hbm, w2_buf, 32 * r2[k], 32))
            seq.append((w1_hbm, w1_buf, 8 * r6[k], 8))
        n_ffn = len(seq)
        seq = [rows(*e, 0 if n < lead + 2 * chunk else 1 if n < lead + 4 * chunk else 2) for n, e in enumerate(seq)]
        for y in range(4):
            seq += [rows(wo_hbm, wo_buf, 32 * (g + 4 * y), 32, 3 + y) for g in _order(ob) if (g + 4 * y) // 4 not in VH]
        t0 = seq[:lead] + seq[lead + 1::2]
        t1 = seq[lead::2]
        vrows = [h * D + r for h in VH for r in range(0, D, tiny)]
        ends = [sum(vpu[:i + 1]) for i in range(len(vpu))]
        for n, r in enumerate(vrows):
            t1.append(rows(wo_hbm, wo_buf, r, tiny, 7 + sum(n * tiny >= e for e in ends)))

        def start_tail(c, last=False):
            for k in range(c * chunk, max(len(t0), len(t1)) if last else (c + 1) * chunk):
                for t, p in ((t0, 0), (t1, 1)):
                    if k < len(t):
                        copy(t[k][0], t[k][1], tsems.at[t[k][2]]).start(priority=p)

        def wait_tail(s):
            for e in t0 + t1:
                if e[2] == s:
                    copy(e[0], e[1], tsems.at[s]).wait()

        x_copy = copy(x_hbm, x_buf, sem_small.at[0])
        b1_copy = copy(b1_hbm, b1_buf, sem_small.at[1])
        b2_copy = copy(b2_hbm, b2_buf, sem_small.at[1])
        start_weight(wq_hbm, wq_buf, 0, 0, first)
        x_copy.start()
        b1_copy.start()
        b2_copy.start()
        pl.loop(1, AHEAD)(lambda y: start_weight(wq_hbm, wq_buf, y, y))

        x_copy.wait()
        x = x_buf[...].astype(F32)
        xc = x - jnp.mean(x, axis=-1, keepdims=True)
        var = jnp.mean(xc * xc, axis=-1, keepdims=True)
        xn = (xc * lax.rsqrt(var + 1e-5)).astype(BF16)
        xp = jnp.concatenate([xn.astype(F32), jnp.zeros((128 - B, M), F32)], axis=0)
        for j in range(M // 128):
            xt = xp[:, j * 128:(j + 1) * 128].T
            for b in range(B):
                xb_ref[b, j * 128:(j + 1) * 128, :] = jnp.broadcast_to(xt[:, b:b + 1], (128, 128))

        def q_slot(y, carry):
            mark('q_ready')
            wait_all(wq_buf.at[y], sems.at[y])
            mark('q_arr')
            pl.when(y == 0)(lambda: start_weight(wq_hbm, wq_buf, AHEAD, AHEAD))
            pl.when(y > 0)(lambda: start_weight(wuk_hbm, wuk_buf, y - 1, y + AHEAD))

            def q_body(t, carry):
                q0, q1 = carry
                for v in range(2):
                    i, u = t // 4, (t % 4) * 2 + v
                    for r in range(4):
                        m = i * 128 + (4 * u + y) * 4 + r
                        w = wq_buf[y, i, u, r].astype(F32)
                        q0 = q0 + xb_ref[0, pl.ds(m, 1), :] * w
                        q1 = q1 + xb_ref[1, pl.ds(m, 1), :] * w
                return q0, q1

            return lax.fori_loop(0, 16, q_body, carry)

        q01 = lax.fori_loop(0, 4, q_slot, (jnp.zeros((H, D), F32), jnp.zeros((H, D), F32)))
        q = jnp.concatenate([q01[0], q01[1], jnp.zeros((128 - B * H, D), F32)], axis=0).astype(BF16)

        group = (lax.broadcasted_iota(jnp.int32, (16, 8, 128), 2) % H) // 8

        @pl.loop(0, 4)
        def _(y):
            mark('k_ready')
            wait_all(wuk_buf.at[y], sems.at[y])
            mark('k_arr')
            pl.when(y == 0)(lambda: start_weight(wuk_hbm, wuk_buf, AHEAD, AHEAD))
            pl.when(y > 0)(lambda: start_ckv(y - 1))

            @pl.loop(0, 8, unroll=QU)
            def _(s):
                i, u0 = s // 2, (s % 2) * 4
                w = wuk_buf[y, i, pl.ds(u0, 4)].reshape(16 * H, D)
                r = lax.dot_general(w, q, NT, preferred_element_type=F32).reshape(16, 4, 8, 128)
                v = jnp.where(group == 0, r[:, 0],
                              jnp.where(group == 1, r[:, 1], jnp.where(group == 2, r[:, 2], r[:, 3])))
                for u in range(4):
                    o = (i * 32 + 4 * (u0 + u) + y) * 32
                    t8[pl.ds(pl.multiple_of(o, 32), 32), :] = v[4 * u:4 * u + 4].reshape(32, 128)

        sub = lax.broadcasted_iota(jnp.int32, (128, 128), 1) % 8
        for j in range(DC // 128):
            t = t8[pl.ds(j * 1024, 128, stride=8), :]
            for s in range(1, 8):
                t = jnp.where(sub == s, t8[pl.ds(j * 1024 + s, 128, stride=8), :], t)
            qa_ref[:, j * 128:(j + 1) * 128] = (t.T[:B * H] * (D ** -0.5 * LOG2E)).astype(BF16)

        m_ref[...] = jnp.full((B * H, 128), -jnp.inf, F32)
        l_ref[...] = jnp.zeros((B * H, 128), F32)
        acc_ref[...] = jnp.zeros((B * H, DC), F32)

        @pl.loop(0, NCB)
        def _(i):
            mark('c_ready')
            wait_all(c_buf.at[i], sems.at[i % NS])
            mark('c_arr')
            pl.when(i + AHEAD < NCB)(lambda: start_ckv(i + AHEAD))
            pl.when(i + AHEAD >= NCB)(lambda: start_weight(wuv_hbm, wuv_buf, i + AHEAD - NCB, i + AHEAD))
            if noatt:
                return
            hrows = pl.ds(pl.multiple_of((i // (NCB // B)) * H, H), H)
            c = c_buf[i].reshape(1024, DC)
            sc = lax.dot_general(qa_ref[hrows, :], c, NT, preferred_element_type=F32)
            m_prev = m_ref[hrows, :]
            m_new = jnp.maximum(m_prev, jnp.max(sc, axis=1, keepdims=True))
            p = jnp.exp2(sc - m_new[:, :1])
            alpha = jnp.exp2(m_prev - m_new)
            l_ref[hrows, :] = alpha * l_ref[hrows, :] + jnp.sum(p, axis=1, keepdims=True)
            m_ref[hrows, :] = m_new
            pv = jnp.dot(p.astype(BF16), c, preferred_element_type=F32)
            acc_ref[hrows, :] = acc_ref[hrows, :] * alpha[:, :1] + pv

        pc = (acc_ref[...] / l_ref[...][:, :1]).astype(BF16)
        pcs = jnp.concatenate([pc[:, j * 128:(j + 1) * 128] for j in range(DC // 128)], axis=0)
        lane = lax.broadcasted_iota(jnp.int32, (4 * B * H, 128), 1)
        diag = (lane % H) == lax.broadcasted_iota(jnp.int32, (4 * B * H, 128), 0) % H
        src = lax.broadcasted_iota(jnp.int32, (128, 128), 0) - lax.broadcasted_iota(jnp.int32, (128, 128), 1) // H

        def v_slot(y, ctx):
            @pl.loop(0, 8, unroll=4)
            def _(u):
                rep = jnp.dot(pcs, jnp.where(src == 4 * (4 * u + y), 1.0, 0.0).astype(BF16), preferred_element_type=F32)
                a_buf[:, u] = jnp.where(diag, rep, 0.0).astype(BF16).reshape(4, B * H, 128)

            mark('v_ready')
            wait_all(wuv_buf.at[y], sems.at[y])
            mark('v_arr')
            pl.when(y == 0)(lambda: start_weight(wuv_hbm, wuv_buf, AHEAD, AHEAD))
            for c in range(AHEAD):
                pl.when(y == c + 1)(lambda c=c: start_tail(c))
            lhs = jnp.concatenate([a_buf[i, u] for i in range(4) for u in range(8)], axis=1)
            return ctx + jnp.dot(lhs, wuv_buf[y].reshape(128 * H, D), preferred_element_type=F32)

        ctx_ref[...] = lax.fori_loop(0, 4, v_slot, jnp.zeros((B * H, D), F32))

        def ctx_heads(hs):
            v = jnp.concatenate([ctx_ref[pl.ds(h, B, stride=H), :] for h in hs], axis=1)
            return jnp.concatenate([v, jnp.zeros((8 - B, v.shape[1]), F32)], axis=0).astype(BF16)

        for t, hh in enumerate(VH):
            ct = jnp.concatenate([ctx_ref[pl.ds(hh, B, stride=H), :], jnp.zeros((128 - B, D), F32)], axis=0).T
            for b in range(B):
                cb_ref[b, pl.ds(t * D, D), :] = jnp.broadcast_to(ct[:, b:b + 1], (D, 128))

        b1_copy.wait()
        b2_copy.wait()
        for s in range(3):
            mark('f_ready')
            wait_tail(s)
            mark('f_arr')
            start_tail(AHEAD + s)
        xn8 = jnp.concatenate([xn.astype(F32), jnp.zeros((8 - B, M), F32)], axis=0).astype(BF16)
        h = jnp.dot(xn8, w1_buf[...], preferred_element_type=F32) + b1_buf[...].astype(F32).reshape(1, F)
        h = jax.nn.gelu(h, approximate=True).astype(BF16)
        gg = jnp.dot(h, w2_buf[...], preferred_element_type=F32) + b2_buf[...].astype(F32).reshape(1, M)
        gate = gg * jax.nn.sigmoid(gg)

        s = jnp.zeros((8, M), F32)
        for y in range(4):
            hs = [hh for hh in range(y, H, 4) if hh not in VH]
            lhs = ctx_heads(hs)
            mark('o_ready')
            wait_tail(3 + y)
            mark('o_arr')
            if y < 3:
                start_tail(AHEAD + 3 + y, last=y == 2)
            w = jnp.concatenate([wo_buf[pl.ds(hh * D, D), :] for hh in hs], axis=0)
            s = s + jnp.dot(lhs, w, preferred_element_type=F32)
        base = jnp.concatenate([x, jnp.zeros((8 - B, M), F32)], axis=0) + s * gate
        acc = [None] * B
        o = 0
        for i, n in enumerate(vpu):
            mark('t_ready')
            v = wo_buf.at[pl.ds(0, n)]
            wait_all(v, tsems.at[7 + i])
            mark('t_arr')
            for r0 in range(o, o + n, 8):
                w = wo_buf[pl.ds(VH[r0 // D] * D + r0 % D, 8), :].astype(F32)
                for b in range(B):
                    t = w * jnp.concatenate([cb_ref[b, pl.ds(r0, 8), :]] * (M // 128), axis=1)
                    acc[b] = t if acc[b] is None else acc[b] + t
            o += n
        row = lax.broadcasted_iota(jnp.int32, (8, M), 0)
        r = [jnp.sum(acc[b], axis=0, keepdims=True) for b in range(B)]
        o_ref[...] = (base + jnp.where(row == 0, r[0], r[1]) * gate).astype(BF16)[:B]

    def fn(A_x, A_c_kv, A_w_q, A_w_uk, A_w_uv, A_w_o, B_x, B_w1, B_b1, B_w2, B_b2):
        del B_x
        W = (128, 4, H, D)
        WB = (4, 4, 8, 4, H, D)
        out = pl.pallas_call(
            kernel,
            out_shape=jax.ShapeDtypeStruct((B, M), BF16),
            in_specs=[pl.BlockSpec(memory_space=pltpu.HBM)] * 10,
            out_specs=pl.BlockSpec(memory_space=pltpu.VMEM),
            scratch_shapes=[
                pltpu.VMEM((B, M), BF16), pltpu.VMEM((F,), BF16), pltpu.VMEM((M,), BF16),
                pltpu.VMEM((NCB, 32, 32, DC), BF16),
                pltpu.VMEM(WB, BF16), pltpu.VMEM(WB, BF16), pltpu.VMEM(WB, BF16),
                pltpu.VMEM((H * D, M), BF16), pltpu.VMEM((M, F), BF16), pltpu.VMEM((F, M), BF16),
                pltpu.VMEM((B, M, 128), F32),
                pltpu.VMEM((DC * 8 + 8, 128), F32),
                pltpu.VMEM((B * H, DC), BF16), pltpu.VMEM((B * H, DC), F32),
                pltpu.VMEM((B * H, 128), F32), pltpu.VMEM((B * H, 128), F32),
                pltpu.VMEM((4, 8, B * H, 128), BF16), pltpu.VMEM((B * H, D), F32),
                pltpu.VMEM((B, len(VH) * D, 128), F32),
                pltpu.SemaphoreType.DMA((NS,)), pltpu.SemaphoreType.DMA((7 + len(vpu),)), pltpu.SemaphoreType.DMA((2,)),
            ],
            compiler_params=pltpu.CompilerParams(vmem_limit_bytes=100 * 1024 * 1024, disable_bounds_checks=True,
                                                 disable_semaphore_checks=True, flags=flags),
        )(A_x.reshape(B, M), A_c_kv.reshape(B * SK // 32, 32, DC), A_w_q.reshape(W), A_w_uk.reshape(W), A_w_uv.reshape(W),
          A_w_o.reshape(H * D, M), B_w1, B_b1, B_w2, B_b2)
        return out.reshape(B, 1, M)
    return fn


_impl = make_kernel(**dict())


@jax.jit
def pallas_recurrent_scan__compressed_kv_cla__dense_activation_gelu__decode_kernel(
    A_x: jax.Array,
    A_c_kv: jax.Array,
    A_w_q: jax.Array,
    A_w_uk: jax.Array,
    A_w_uv: jax.Array,
    A_w_o: jax.Array,
    B_x: jax.Array,
    B_w1: jax.Array,
    B_b1: jax.Array,
    B_w2: jax.Array,
    B_b2: jax.Array,
):
    return _impl(A_x, A_c_kv, A_w_q, A_w_uk, A_w_uv, A_w_o, B_x, B_w1, B_b1, B_w2, B_b2)
```

```python
import jax
import jax.numpy as jnp
from jax import lax
import jax.experimental.pallas as pl
import jax.experimental.pallas.tpu as pltpu

F32 = jnp.float32
BF16 = jnp.bfloat16
B, H, SK, D, M, DC, F = 2, 32, 16384, 128, 512, 512, 1792
LOG2E = 1.4426950408889634
NT = (((1,), (1,)), ((), ()))


def _order(bits):
    return [sum(((c >> k) & 1) << b for k, b in enumerate(bits)) for c in range(1 << len(bits))]


def make_kernel(wb=(4, 5, 6, 0, 1), cb=(5, 6, 7, 8, 0), ob=(4, 5, 6, 0, 1), lead=27, vpu=(128, 64, 32, 32), tiny=8,
                QU=4, f1=(5, 4, 3, 2, 1, 0), f2=(5, 4, 3, 2, 1, 0), fmix=True, flip=0, ex=8, flags=None, prof=False, noatt=False):
    def mark(name):
        if prof:
            with jax.named_scope(name):
                pl.delay(1)

    AHEAD = 3
    NS = 8
    NCB = 32
    VH = (27, 31)
    assert sum(vpu) == len(VH) * D

    def kernel(x_hbm, ckv_hbm, wq_hbm, wuk_hbm, wuv_hbm, wo_hbm, w1_hbm, b1_hbm, w2_hbm, b2_hbm,
               o_ref,
               x_buf, b1_buf, b2_buf, c_buf, wq_buf, wuk_buf, wuv_buf, wo_buf, w1_buf, w2_buf,
               xb_ref, t8, qa_ref, acc_ref, m_ref, l_ref, a_buf, ctx_ref, cb_ref, sems, tsems, sem_small):
        def copy(src, dst, sem):
            return pltpu.make_async_copy(src, dst, sem)

        def wait_all(buf, sem):
            copy(buf, buf, sem).wait()

        wfree = [b for b in range(7) if b not in wb]
        cfree = [b for b in range(10) if b not in cb]
        wcols = [b for b in range(5) if b in wb]
        word, cord = _order(wb), _order(cb)

        def spread_bits(v, bits):
            return sum(((v >> k) & 1) << b for k, b in enumerate(bits))

        def col(y, u):
            return spread_bits(y, wfree) + spread_bits(u, wcols)

        def rows(hbm, buf, o, n, s):
            return (hbm.at[pl.ds(o, n)], buf.at[pl.ds(o, n)], tsems.at[s], s)

        a1 = [(w1_hbm, w1_buf, 8 * g, 8) for g in _order(f1)]
        a2 = [(w2_hbm, w2_buf, 32 * g, 32) for g in _order(f2) if g < F // 32]
        tail = [e for k in range(64) for e in a2[k:k + 1] + [a1[k]]] if fmix else a1 + a2
        tail = [rows(*e, n // 32) for n, e in enumerate(tail)]
        for y in range(4):
            tail += [rows(wo_hbm, wo_buf, 32 * (g + 4 * y), 32, 4 + y) for g in _order(ob) if (g + 4 * y) // 4 not in VH]
        ends = [sum(vpu[:i + 1]) for i in range(len(vpu))]
        last = [rows(wo_hbm, wo_buf, VH[r // D] * D + r % D, tiny, 8 + sum(r >= e for e in ends)) for r in range(0, len(VH) * D, tiny)]
        n_pairs = 44 * 16 + len(tail) // 2

        def item(blk, pos):
            if isinstance(blk, int) and blk >= 44:
                return tail[(blk - 44) * 32 + pos][:3]
            if isinstance(blk, int) and not 8 <= blk < 40:
                hbm, buf = (wq_hbm, wq_buf) if blk < 4 else (wuk_hbm, wuk_buf) if blk < 8 else (wuv_hbm, wuv_buf)
                y, g = blk % 4, word[pos]
                u = sum(((g >> b) & 1) << k for k, b in enumerate(wcols))
                return hbm.at[spread_bits(y, wfree) + g], buf.at[y, g // 32, u], sems.at[blk % NS]
            return ckv_hbm.at[spread_bits(blk - 8, cfree) + cord[pos]], c_buf.at[blk - 8, pos], sems.at[blk % NS]

        def issue(lo, hi):
            for k in range(lo, hi):
                if 0 <= k - lead < n_pairs:
                    copy(*item((k - lead) // 16, 2 * ((k - lead) % 16) + flip)).start(priority=0)
                if k < n_pairs:
                    copy(*item(k // 16, 2 * (k % 16) + 1 - flip)).start(priority=1)
                elif k - n_pairs < len(last):
                    copy(*last[k - n_pairs][:3]).start(priority=1)

        def issue_slot(t):
            if isinstance(t, int):
                return issue(16 * t + ex, 16 * t + 16 + ex)
            for m in range(ex, 16 + ex):
                copy(*item(t + (m - lead) // 16, 2 * ((m - lead) % 16) + flip)).start(priority=0)
                copy(*item(t + m // 16, 2 * (m % 16) + 1 - flip)).start(priority=1)

        def wait_tail(s):
            for e in tail + last:
                if e[3] == s:
                    copy(*e[:3]).wait()

        x_copy = copy(x_hbm, x_buf, sem_small.at[0])
        b1_copy = copy(b1_hbm, b1_buf, sem_small.at[1])
        b2_copy = copy(b2_hbm, b2_buf, sem_small.at[1])
        x_copy.start()
        issue(0, 40)
        b1_copy.start()
        b2_copy.start()
        x_copy.wait()
        issue(40, 48 + ex)

        x = x_buf[...].astype(F32)
        xc = x - jnp.mean(x, axis=-1, keepdims=True)
        var = jnp.mean(xc * xc, axis=-1, keepdims=True)
        xn = (xc * lax.rsqrt(var + 1e-5)).astype(BF16)
        xp = jnp.concatenate([xn.astype(F32), jnp.zeros((128 - B, M), F32)], axis=0)
        for j in range(M // 128):
            xt = xp[:, j * 128:(j + 1) * 128].T
            for b in range(B):
                xb_ref[b, j * 128:(j + 1) * 128, :] = jnp.broadcast_to(xt[:, b:b + 1], (128, 128))

        def q_slot(y, carry):
            mark('q_ready')
            wait_all(wq_buf.at[y], sems.at[y])
            mark('q_arr')
            for t in range(4):
                pl.when(y == t)(lambda t=t: issue_slot(t + AHEAD))

            def q_body(t, carry):
                q0, q1 = carry
                for v in range(2):
                    i, u = t // 4, (t % 4) * 2 + v
                    for r in range(4):
                        m = i * 128 + col(y, u) * 4 + r
                        w = wq_buf[y, i, u, r].astype(F32)
                        q0 = q0 + xb_ref[0, pl.ds(m, 1), :] * w
                        q1 = q1 + xb_ref[1, pl.ds(m, 1), :] * w
                return q0, q1

            return lax.fori_loop(0, 16, q_body, carry)

        q01 = lax.fori_loop(0, 4, q_slot, (jnp.zeros((H, D), F32), jnp.zeros((H, D), F32)))
        q = jnp.concatenate([q01[0], q01[1], jnp.zeros((128 - B * H, D), F32)], axis=0).astype(BF16)

        group = (lax.broadcasted_iota(jnp.int32, (16, 8, 128), 2) % H) // 8

        @pl.loop(0, 4)
        def _(y):
            mark('k_ready')
            wait_all(wuk_buf.at[y], sems.at[y + 4])
            mark('k_arr')
            for t in range(4):
                pl.when(y == t)(lambda t=t: issue_slot(t + 4 + AHEAD))

            @pl.loop(0, 8, unroll=QU)
            def _(s):
                i, u0 = s // 2, (s % 2) * 4
                w = wuk_buf[y, i, pl.ds(u0, 4)].reshape(16 * H, D)
                r = lax.dot_general(w, q, NT, preferred_element_type=F32).reshape(16, 4, 8, 128)
                v = jnp.where(group == 0, r[:, 0],
                              jnp.where(group == 1, r[:, 1], jnp.where(group == 2, r[:, 2], r[:, 3])))
                for u in range(4):
                    o = (i * 32 + col(y, u0 + u)) * 32
                    t8[pl.ds(pl.multiple_of(o, 32), 32), :] = v[4 * u:4 * u + 4].reshape(32, 128)

        sub = lax.broadcasted_iota(jnp.int32, (128, 128), 1) % 8
        for j in range(DC // 128):
            t = t8[pl.ds(j * 1024, 128, stride=8), :]
            for s in range(1, 8):
                t = jnp.where(sub == s, t8[pl.ds(j * 1024 + s, 128, stride=8), :], t)
            qa_ref[:, j * 128:(j + 1) * 128] = (t.T[:B * H] * (D ** -0.5 * LOG2E)).astype(BF16)

        m_ref[...] = jnp.full((B * H, 128), -jnp.inf, F32)
        l_ref[...] = jnp.zeros((B * H, 128), F32)
        acc_ref[...] = jnp.zeros((B * H, DC), F32)

        @pl.loop(0, NCB)
        def _(i):
            mark('c_ready')
            wait_all(c_buf.at[i], sems.at[i % NS])
            mark('c_arr')
            dyn = NCB - AHEAD - (ex > 0)
            pl.when(i < dyn)(lambda: issue_slot(i + 8 + AHEAD))
            for t in range(dyn, NCB):
                pl.when(i == t)(lambda t=t: issue_slot(t + 8 + AHEAD))
            if noatt:
                return
            hrows = pl.ds(pl.multiple_of((i // (NCB // B)) * H, H), H)
            c = c_buf[i].reshape(1024, DC)
            sc = lax.dot_general(qa_ref[hrows, :], c, NT, preferred_element_type=F32)
            m_prev = m_ref[hrows, :]
            m_new = jnp.maximum(m_prev, jnp.max(sc, axis=1, keepdims=True))
            p = jnp.exp2(sc - m_new[:, :1])
            alpha = jnp.exp2(m_prev - m_new)
            l_ref[hrows, :] = alpha * l_ref[hrows, :] + jnp.sum(p, axis=1, keepdims=True)
            m_ref[hrows, :] = m_new
            pv = jnp.dot(p.astype(BF16), c, preferred_element_type=F32)
            acc_ref[hrows, :] = acc_ref[hrows, :] * alpha[:, :1] + pv

        pc = (acc_ref[...] / l_ref[...][:, :1]).astype(BF16)
        pcs = jnp.concatenate([pc[:, j * 128:(j + 1) * 128] for j in range(DC // 128)], axis=0)
        lane = lax.broadcasted_iota(jnp.int32, (4 * B * H, 128), 1)
        diag = (lane % H) == lax.broadcasted_iota(jnp.int32, (4 * B * H, 128), 0) % H
        src = lax.broadcasted_iota(jnp.int32, (128, 128), 0) - lax.broadcasted_iota(jnp.int32, (128, 128), 1) // H

        def v_slot(y, ctx):
            @pl.loop(0, 8, unroll=4)
            def _(u):
                rep = jnp.dot(pcs, jnp.where(src == 4 * col(y, u), 1.0, 0.0).astype(BF16), preferred_element_type=F32)
                a_buf[:, u] = jnp.where(diag, rep, 0.0).astype(BF16).reshape(4, B * H, 128)

            mark('v_ready')
            wait_all(wuv_buf.at[y], sems.at[y])
            mark('v_arr')
            for t in range(4):
                pl.when(y == t)(lambda t=t: issue_slot(t + 40 + AHEAD))
            lhs = jnp.concatenate([a_buf[i, u] for i in range(4) for u in range(8)], axis=1)
            return ctx + jnp.dot(lhs, wuv_buf[y].reshape(128 * H, D), preferred_element_type=F32)

        ctx_ref[...] = lax.fori_loop(0, 4, v_slot, jnp.zeros((B * H, D), F32))

        def ctx_heads(hs):
            v = jnp.concatenate([ctx_ref[pl.ds(h, B, stride=H), :] for h in hs], axis=1)
            return jnp.concatenate([v, jnp.zeros((8 - B, v.shape[1]), F32)], axis=0).astype(BF16)

        for t, hh in enumerate(VH):
            ct = jnp.concatenate([ctx_ref[pl.ds(hh, B, stride=H), :], jnp.zeros((128 - B, D), F32)], axis=0).T
            for b in range(B):
                cb_ref[b, pl.ds(t * D, D), :] = jnp.broadcast_to(ct[:, b:b + 1], (D, 128))

        b1_copy.wait()
        b2_copy.wait()
        done = 16 * 47 + ex
        for s in range(4):
            mark('f_ready')
            wait_tail(s)
            mark('f_arr')
            issue(done, done + (16 if s < 3 else 12))
            done += 16 if s < 3 else 12
        xn8 = jnp.concatenate([xn.astype(F32), jnp.zeros((8 - B, M), F32)], axis=0).astype(BF16)
        h = jnp.dot(xn8, w1_buf[...], preferred_element_type=F32) + b1_buf[...].astype(F32).reshape(1, F)
        h = jax.nn.gelu(h, approximate=True).astype(BF16)
        gg = jnp.dot(h, w2_buf[...], preferred_element_type=F32) + b2_buf[...].astype(F32).reshape(1, M)
        gate = gg * jax.nn.sigmoid(gg)

        s = jnp.zeros((8, M), F32)
        for y in range(4):
            hs = [hh for hh in range(y, H, 4) if hh not in VH]
            lhs = ctx_heads(hs)
            mark('o_ready')
            wait_tail(4 + y)
            mark('o_arr')
            if y < 3:
                issue(done, done + 16 if y < 2 else n_pairs + max(lead, len(last)))
                done += 16
            w = jnp.concatenate([wo_buf[pl.ds(hh * D, D), :] for hh in hs], axis=0)
            s = s + jnp.dot(lhs, w, preferred_element_type=F32)
        base = jnp.concatenate([x, jnp.zeros((8 - B, M), F32)], axis=0) + s * gate
        acc = [None] * B
        o = 0
        for i, n in enumerate(vpu):
            mark('t_ready')
            v = wo_buf.at[pl.ds(0, n)]
            wait_all(v, tsems.at[8 + i])
            mark('t_arr')
            for r0 in range(o, o + n, 8):
                w = wo_buf[pl.ds(VH[r0 // D] * D + r0 % D, 8), :].astype(F32)
                for b in range(B):
                    t = w * jnp.concatenate([cb_ref[b, pl.ds(r0, 8), :]] * (M // 128), axis=1)
                    acc[b] = t if acc[b] is None else acc[b] + t
            o += n
        row = lax.broadcasted_iota(jnp.int32, (8, M), 0)
        r = [jnp.sum(acc[b], axis=0, keepdims=True) for b in range(B)]
        o_ref[...] = (base + jnp.where(row == 0, r[0], r[1]) * gate).astype(BF16)[:B]

    def fn(A_x, A_c_kv, A_w_q, A_w_uk, A_w_uv, A_w_o, B_x, B_w1, B_b1, B_w2, B_b2):
        del B_x
        W = (128, 4, H, D)
        WB = (4, 4, 8, 4, H, D)
        out = pl.pallas_call(
            kernel,
            out_shape=jax.ShapeDtypeStruct((B, M), BF16),
            in_specs=[pl.BlockSpec(memory_space=pltpu.HBM)] * 10,
            out_specs=pl.BlockSpec(memory_space=pltpu.VMEM),
            scratch_shapes=[
                pltpu.VMEM((B, M), BF16), pltpu.VMEM((F,), BF16), pltpu.VMEM((M,), BF16),
                pltpu.VMEM((NCB, 32, 32, DC), BF16),
                pltpu.VMEM(WB, BF16), pltpu.VMEM(WB, BF16), pltpu.VMEM(WB, BF16),
                pltpu.VMEM((H * D, M), BF16), pltpu.VMEM((M, F), BF16), pltpu.VMEM((F, M), BF16),
                pltpu.VMEM((B, M, 128), F32),
                pltpu.VMEM((DC * 8 + 8, 128), F32),
                pltpu.VMEM((B * H, DC), BF16), pltpu.VMEM((B * H, DC), F32),
                pltpu.VMEM((B * H, 128), F32), pltpu.VMEM((B * H, 128), F32),
                pltpu.VMEM((4, 8, B * H, 128), BF16), pltpu.VMEM((B * H, D), F32),
                pltpu.VMEM((B, len(VH) * D, 128), F32),
                pltpu.SemaphoreType.DMA((NS,)), pltpu.SemaphoreType.DMA((8 + len(vpu),)), pltpu.SemaphoreType.DMA((2,)),
            ],
            compiler_params=pltpu.CompilerParams(vmem_limit_bytes=100 * 1024 * 1024, disable_bounds_checks=True,
                                                 disable_semaphore_checks=True, flags=flags),
        )(A_x.reshape(B, M), A_c_kv.reshape(B * SK // 32, 32, DC), A_w_q.reshape(W), A_w_uk.reshape(W), A_w_uv.reshape(W),
          A_w_o.reshape(H * D, M), B_w1, B_b1, B_w2, B_b2)
        return out.reshape(B, 1, M)
    return fn


_impl = make_kernel(**dict(lead=26))


@jax.jit
def pallas_recurrent_scan__compressed_kv_cla__dense_activation_gelu__decode_kernel(
    A_x: jax.Array,
    A_c_kv: jax.Array,
    A_w_q: jax.Array,
    A_w_uk: jax.Array,
    A_w_uv: jax.Array,
    A_w_o: jax.Array,
    B_x: jax.Array,
    B_w1: jax.Array,
    B_b1: jax.Array,
    B_w2: jax.Array,
    B_b2: jax.Array,
):
    return _impl(A_x, A_c_kv, A_w_q, A_w_uk, A_w_uv, A_w_o, B_x, B_w1, B_b1, B_w2, B_b2)
```

```python
import jax
import jax.numpy as jnp
from jax import lax
import jax.experimental.pallas as pl
import jax.experimental.pallas.tpu as pltpu

F32 = jnp.float32
BF16 = jnp.bfloat16
B, H, SK, D, M, DC, F = 2, 32, 16384, 128, 512, 512, 1792
LOG2E = 1.4426950408889634
NT = (((1,), (1,)), ((), ()))


def make_kernel(lead=26, ex=8, vpu=(128, 64, 32, 32), tiny=8, QU=4, IU=4, NM=5, NT0=6, vs=0, first=40, cs=5, ffn=0, flags=None, nocomp=False, wmode=0, prof=False):
    def mark(name):
        if prof:
            with jax.named_scope(name):
                pl.delay(1)

    NS = 8
    NCB = 32
    assert sum(vpu) == (8 - NT0) * D
    NV = NT0 - NM

    def kernel(x_hbm, ckv_hbm, wq_hbm, wuk_hbm, wuv_hbm, wo_hbm, w1_hbm, b1_hbm, w2_hbm, b2_hbm,
               o_ref,
               x_buf, b1_buf, b2_buf, c_buf, wq_buf, wuk_buf, wuv_buf, wo_buf, w1_buf, w2_buf,
               xb_ref, t8, qa_ref, acc_ref, m_ref, l_ref, a_buf, ctx_ref, cb_ref, sems, tsems, sem_small):
        def copy(src, dst, sem):
            return pltpu.make_async_copy(src, dst, sem)

        def wait_all(buf, sem):
            copy(buf, buf, sem).wait()

        def aligned(o, n):
            return pl.ds(o if isinstance(o, int) else pl.multiple_of(o, n), n)

        def weight(hbm, buf, slot):
            def f(n, e):
                p = 2 * n + e
                y, r, c = p >> 5, p & 7, (p >> 3) & 3
                return copy(hbm.at[16 * r + 4 * y + c], buf.at[y, r, c], sems.at[slot + y])
            return f

        def ckv(n, e):
            p = 2 * n + e
            y = p >> 5
            r, c = p & ((512 >> cs) - 1), (p & 511) >> (9 - cs)
            return copy(ckv_hbm.at[(p & 512) + (r << cs) + c], c_buf.at[y, p & 31], sems.at[y & (NS - 1)])

        def w1_piece(g, n):
            r = aligned(8 * g, 8)
            return copy(w1_hbm.at[r], w1_buf.at[r], tsems.at[n >> 4])

        def ffn_a(n, e):
            r, c = n & 7, n >> 3
            r = ((r & 1) << 2) | (r & 2) | (r >> 2)
            if e == ffn:
                g = 7 * r + c
                return copy(w2_hbm.at[aligned(32 * g, 32)], w2_buf.at[aligned(32 * g, 32)], tsems.at[n >> 4])
            return w1_piece(8 * r + c, n)

        def ffn_b(n, e):
            return w1_piece(8 * (n + 4 * e) + 7, 56)

        def wo_a(n, e):
            p = 2 * n + e
            y, r, c = p >> 5, p & 7, (p >> 3) & 3
            return copy(wo_hbm.at[16 * r + 4 * y + c], wo_buf.at[y, r, c], tsems.at[4 + y])

        def wo_b(r0, nr, s0, split):
            def f(n, e):
                p = 2 * n + e
                c = (p * (256 // nr + 1)) >> 8
                r = r0 + p - nr * c
                return copy(wo_hbm.at[16 * r + 12 + c], wo_buf.at[3, r, c], tsems.at[s0 + (c >> (2 - split))])
            return f

        per = 32 // tiny
        ends = [sum(vpu[:i + 1]) // tiny for i in range(len(vpu))]

        def last(i):
            def f(n, e):
                n = n + ([0] + ends)[i]
                r, c, o = NT0 + n // (4 * per), (n // per) & 3, aligned((n % per) * tiny, tiny)
                return copy(wo_hbm.at[16 * r + 12 + c, o], wo_buf.at[3, r, c, o], tsems.at[8 + i])
            return f

        segs = [(64, weight(wq_hbm, wq_buf, 0)), (64, weight(wuk_hbm, wuk_buf, 4)), (512, ckv), (64, weight(wuv_hbm, wuv_buf, 0)),
                (56, ffn_a), (4, ffn_b), (48, wo_a), (2 * NM, wo_b(0, NM, 7, 0))] + ([(2 * NV, wo_b(NM, NV, 8 + len(vpu), vs))] if NV else [])
        n_pairs = sum(n for n, _ in segs)
        segs1 = segs + [(n // tiny, last(i)) for i, n in enumerate(vpu)]

        def find(segs, k):
            o = 0
            for n, f in segs:
                if o <= k < o + n:
                    return o, o + n, f
                o += n
            return 0, 0 if k < 0 else 1 << 30, None

        def issue(lo, hi):
            while lo < hi:
                o0, e0, f0 = find(segs, lo - lead)
                o1, e1, f1 = find(segs1, lo)
                e = min(hi, e0 + lead, e1)

                @pl.loop(lo, e, unroll=IU)
                def _(k):
                    if f0:
                        f0(k - (lead + o0), 0).start(priority=0)
                    if f1:
                        f1(k - o1, 1).start(priority=1)
                lo = e

        def top_up(blk):
            issue(16 * (blk + 3) + ex, 16 * (blk + 4) + ex)

        x_copy = copy(x_hbm, x_buf, sem_small.at[0])
        b1_copy = copy(b1_hbm, b1_buf, sem_small.at[1])
        b2_copy = copy(b2_hbm, b2_buf, sem_small.at[1])
        issue(0, 1)
        x_copy.start()
        b1_copy.start()
        b2_copy.start()
        issue(1, first)

        if nocomp:
            x_copy.wait(); b1_copy.wait(); b2_copy.wait()
            issue(first, n_pairs + max(lead, ends[-1]))
            for y in range(4):
                for buf, sl in ((wq_buf, y), (wuk_buf, y + 4), (wuv_buf, y)):
                    wait_all(buf.at[y], sems.at[sl])
                wait_all(w1_buf.at[pl.ds(0, 128)], tsems.at[y])
                wait_all(w2_buf.at[pl.ds(0, 512 if y < 3 else 256)], tsems.at[y])
                wait_all(wo_buf.at[y, pl.ds(0, 8 if y < 3 else NM)], tsems.at[4 + y])
            for i in range(8):
                wait_all(c_buf.at[pl.ds(0, 4)], sems.at[i])
            for k in range(1 << vs if NV else 0):
                wait_all(wo_buf.at[3, pl.ds(NM, NV), pl.ds(0, 4 >> vs)], tsems.at[8 + len(vpu) + k])
            for i, n in enumerate(vpu):
                wait_all(w2_buf.at[pl.ds(0, n)], tsems.at[8 + i])
            o_ref[...] = x_buf[...]
            return
        x_copy.wait()
        x = x_buf[...].astype(F32)
        xc = x - jnp.mean(x, axis=-1, keepdims=True)
        var = jnp.mean(xc * xc, axis=-1, keepdims=True)
        xn = (xc * lax.rsqrt(var + 1e-5)).astype(BF16)
        xp = jnp.concatenate([xn.astype(F32), jnp.zeros((128 - B, M), F32)], axis=0)
        for j in range(M // 128):
            xt = xp[:, j * 128:(j + 1) * 128].T
            for b in range(B):
                xb_ref[b, j * 128:(j + 1) * 128, :] = jnp.broadcast_to(xt[:, b:b + 1], (128, 128))
        issue(first, 48 + ex)

        def q_slot(y, carry):
            mark('q_ready')
            wait_all(wq_buf.at[y], sems.at[y])
            mark('q_arr')
            for t in range(4):
                pl.when(y == t)(lambda t=t: top_up(t))

            def q_body(t, carry):
                q0, q1 = carry
                for v in range(8):
                    r, c, e = t >> 1, (t & 1) * 2 + v // 4, v % 4
                    m = (16 * r + 4 * y + c) * 4 + e
                    w = wq_buf[y, r, c, e].astype(F32)
                    q0 = q0 + xb_ref[0, pl.ds(m, 1), :] * w
                    q1 = q1 + xb_ref[1, pl.ds(m, 1), :] * w
                return q0, q1

            return lax.fori_loop(0, 16, q_body, carry)

        q01 = lax.fori_loop(0, 4, q_slot, (jnp.zeros((H, D), F32), jnp.zeros((H, D), F32)))
        q = jnp.concatenate([q01[0], q01[1], jnp.zeros((128 - B * H, D), F32)], axis=0).astype(BF16)

        group = (lax.broadcasted_iota(jnp.int32, (16, 8, 128), 2) % H) // 8

        @pl.loop(0, 4)
        def _(y):
            mark('k_ready')
            wait_all(wuk_buf.at[y], sems.at[y + 4])
            mark('k_arr')
            for t in range(4):
                pl.when(y == t)(lambda t=t: top_up(4 + t))

            @pl.loop(0, 8, unroll=QU)
            def _(r):
                w = wuk_buf[y, r].reshape(16 * H, D)
                v = lax.dot_general(w, q, NT, preferred_element_type=F32).reshape(16, 4, 8, 128)
                v = jnp.where(group == 0, v[:, 0],
                              jnp.where(group == 1, v[:, 1], jnp.where(group == 2, v[:, 2], v[:, 3])))
                t8[aligned((4 * r + y) * 128, 128), :] = v.reshape(128, 128)

        sub = lax.broadcasted_iota(jnp.int32, (128, 128), 1) % 8

        @pl.loop(0, DC // 128)
        def _(j):
            t = t8[pl.ds(j * 1024, 128, stride=8), :]
            for s in range(1, 8):
                t = jnp.where(sub == s, t8[pl.ds(j * 1024 + s, 128, stride=8), :], t)
            qa_ref[j] = (t.T[:B * H] * (D ** -0.5 * LOG2E)).astype(BF16)

        m_ref[...] = jnp.full((B * H, 128), -jnp.inf, F32)
        l_ref[...] = jnp.zeros((B * H, 128), F32)
        acc_ref[...] = jnp.zeros((B * H, DC), F32)

        @pl.loop(0, NCB)
        def _(i):
            mark('c_ready')
            wait_all(c_buf.at[i], sems.at[i & (NS - 1)])
            mark('c_arr')
            inner = NCB - 3 - (ex + 15) // 16

            @pl.when(i < inner)
            def _():
                @pl.loop(0, 16, unroll=IU)
                def _(k):
                    n = 16 * (i + 3) + ex + k
                    ckv(n - lead, 0).start(priority=0)
                    ckv(n, 1).start(priority=1)

            for t in range(inner, NCB):
                pl.when(i == t)(lambda t=t: top_up(8 + t))
            hrows = aligned((i >> 4) * H, H)
            c = c_buf[i].reshape(1024, DC)
            qa = jnp.concatenate([qa_ref[j, hrows, :] for j in range(DC // 128)], axis=1)
            sc = lax.dot_general(qa, c, NT, preferred_element_type=F32)
            m_prev = m_ref[hrows, :]
            m_new = jnp.maximum(m_prev, jnp.max(sc, axis=1, keepdims=True))
            p = jnp.exp2(sc - m_new[:, :1])
            alpha = jnp.exp2(m_prev - m_new)
            l_ref[hrows, :] = alpha * l_ref[hrows, :] + jnp.sum(p, axis=1, keepdims=True)
            m_ref[hrows, :] = m_new
            pv = jnp.dot(p.astype(BF16), c, preferred_element_type=F32)
            acc_ref[hrows, :] = acc_ref[hrows, :] * alpha[:, :1] + pv

        pc = (acc_ref[...] / l_ref[...][:, :1]).astype(BF16)
        pcs = jnp.concatenate([pc[:, j * 128:(j + 1) * 128] for j in range(DC // 128)], axis=0)
        lane = lax.broadcasted_iota(jnp.int32, (4 * B * H, 128), 1)
        diag = (lane % H) == lax.broadcasted_iota(jnp.int32, (4 * B * H, 128), 0) % H
        src = lax.broadcasted_iota(jnp.int32, (128, 128), 0) - lax.broadcasted_iota(jnp.int32, (128, 128), 1) // H

        def v_slot(y, ctx):
            @pl.loop(0, 2)
            def _(u):
                for c in range(4):
                    rep = jnp.dot(pcs, jnp.where(src == 4 * (16 * u + 4 * y + c), 1.0, 0.0).astype(BF16), preferred_element_type=F32)
                    a_buf[:, u, c] = jnp.where(diag, rep, 0.0).astype(BF16).reshape(4, B * H, 128)

            mark('v_ready')
            wait_all(wuv_buf.at[y], sems.at[y])
            mark('v_arr')
            for t in range(4):
                pl.when(y == t)(lambda t=t: top_up(40 + t))
            lhs = jnp.concatenate([a_buf[i, u, c] for i in range(4) for u in range(2) for c in range(4)], axis=1)
            return ctx + jnp.dot(lhs, wuv_buf[y].reshape(128 * H, D), preferred_element_type=F32)

        ctx_ref[...] = lax.fori_loop(0, 4, v_slot, jnp.zeros((B * H, D), F32))

        def ctx_heads(y, n):
            v = jnp.concatenate([ctx_ref[pl.ds(4 * r + y, B, stride=H), :] for r in range(n)], axis=1)
            return jnp.concatenate([v, jnp.zeros((8 - B, n * D), F32)], axis=0).astype(BF16)

        @pl.loop(0, 8 - NM)
        def _(t):
            ct = jnp.concatenate([ctx_ref[pl.ds(4 * (NM + t) + 3, B, stride=H), :], jnp.zeros((128 - B, D), F32)], axis=0).T
            for b in range(B):
                cb_ref[b, aligned(t * D, D), :] = jnp.broadcast_to(ct[:, b:b + 1], (D, 128))

        b1_copy.wait()
        b2_copy.wait()
        for s in range(4):
            mark('f_ready')
            wait_all(w1_buf.at[pl.ds(0, 128)], tsems.at[s])
            wait_all(w2_buf.at[pl.ds(0, 512 if s < 3 else 256)], tsems.at[s])
            mark('f_arr')
            issue(16 * (47 + s) + ex, 16 * (47 + s) + ex + (16 if s < 3 else 12))
        done = 16 * 50 + ex + 12
        xn8 = jnp.concatenate([xn.astype(F32), jnp.zeros((8 - B, M), F32)], axis=0).astype(BF16)
        h = jnp.dot(xn8, w1_buf[...], preferred_element_type=F32) + b1_buf[...].astype(F32).reshape(1, F)
        h = jax.nn.gelu(h, approximate=True).astype(BF16)
        gg = jnp.dot(h, w2_buf[...], preferred_element_type=F32) + b2_buf[...].astype(F32).reshape(1, M)
        gate = gg * jax.nn.sigmoid(gg)

        def o_slot(y, s):
            lhs = ctx_heads(y, 8)
            mark('o_ready')
            wait_all(wo_buf.at[y], tsems.at[4 + y])
            mark('o_arr')
            for t in range(3):
                pl.when(y == t)(lambda t=t: issue(done + 16 * t, done + 16 * t + 16 if t < 2 else n_pairs + max(lead, ends[-1])))
            return s + jnp.dot(lhs, wo_buf[y].reshape(8 * D, M), preferred_element_type=F32)

        s = lax.fori_loop(0, 3, o_slot, jnp.zeros((8, M), F32))
        lhs = ctx_heads(3, NM)
        mark('o_ready')
        wait_all(wo_buf.at[3, pl.ds(0, NM)], tsems.at[7])
        mark('o_arr')
        s = s + jnp.dot(lhs, wo_buf[3, pl.ds(0, NM)].reshape(NM * D, M), preferred_element_type=F32)
        base = jnp.concatenate([x, jnp.zeros((8 - B, M), F32)], axis=0) + s * gate
        acc = [None] * B

        def vpu_rows(r, d):
            w = wo_buf[3, r, d // 32, pl.ds(d % 32, 8), :].astype(F32)
            for b in range(B):
                t = w * jnp.concatenate([cb_ref[b, pl.ds((r - NM) * D + d, 8), :]] * (M // 128), axis=1)
                acc[b] = t if acc[b] is None else acc[b] + t

        for k in range(1 << vs if NV else 0):
            mark('t_ready')
            wait_all(wo_buf.at[3, pl.ds(NM, NV), pl.ds(0, 4 >> vs)], tsems.at[8 + len(vpu) + k])
            mark('t_arr')
            for r in range(NM, NT0):
                for d in range(k * (D >> vs), (k + 1) * (D >> vs), 8):
                    vpu_rows(r, d)
        o = 0
        for i, n in enumerate(vpu):
            mark('t_ready')
            wait_all(w2_buf.at[pl.ds(0, n)], tsems.at[8 + i])
            mark('t_arr')
            for r0 in range(o, o + n, 8):
                vpu_rows(NT0 + r0 // D, r0 % D)
            o += n
        row = lax.broadcasted_iota(jnp.int32, (8, M), 0)
        r = [jnp.sum(acc[b], axis=0, keepdims=True) for b in range(B)]
        o_ref[...] = (base + jnp.where(row == 0, r[0], r[1]) * gate).astype(BF16)[:B]

    def fn(A_x, A_c_kv, A_w_q, A_w_uk, A_w_uv, A_w_o, B_x, B_w1, B_b1, B_w2, B_b2):
        del B_x
        W = (128, 4, H, D)
        WB = (4, 8, 4, 4, H, D)
        out = pl.pallas_call(
            kernel,
            out_shape=jax.ShapeDtypeStruct((B, M), BF16),
            in_specs=[pl.BlockSpec(memory_space=pltpu.HBM)] * 10,
            out_specs=pl.BlockSpec(memory_space=pltpu.VMEM),
            scratch_shapes=[
                pltpu.VMEM((B, M), BF16), pltpu.VMEM((F,), BF16), pltpu.VMEM((M,), BF16),
                pltpu.VMEM((NCB, 32, 32, DC), BF16),
                pltpu.VMEM(WB, BF16), pltpu.VMEM(WB, BF16), pltpu.VMEM(WB, BF16),
                pltpu.VMEM((4, 8, 4, 32, M), BF16), pltpu.VMEM((M, F), BF16), pltpu.VMEM((F, M), BF16),
                pltpu.VMEM((B, M, 128), F32),
                pltpu.VMEM((DC * 8 + 8, 128), F32),
                pltpu.VMEM((DC // 128, B * H, 128), BF16), pltpu.VMEM((B * H, DC), F32),
                pltpu.VMEM((B * H, 128), F32), pltpu.VMEM((B * H, 128), F32),
                pltpu.VMEM((4, 2, 4, B * H, 128), BF16), pltpu.VMEM((B * H, D), F32),
                pltpu.VMEM((B, (8 - NM) * D, 128), F32),
                pltpu.SemaphoreType.DMA((NS,)), pltpu.SemaphoreType.DMA((12 + len(vpu),)), pltpu.SemaphoreType.DMA((2,)),
            ],
            compiler_params=pltpu.CompilerParams(vmem_limit_bytes=100 * 1024 * 1024, disable_bounds_checks=True,
                                                 disable_semaphore_checks=True, flags=flags),
        )(A_x.reshape(B, M), A_c_kv.reshape(B * SK // 32, 32, DC), A_w_q.reshape(W), A_w_uk.reshape(W), A_w_uv.reshape(W),
          A_w_o.reshape(H * D // 32, 32, M), B_w1, B_b1, B_w2, B_b2)
        return out.reshape(B, 1, M)
    return fn


_impl = make_kernel(**dict())


@jax.jit
def pallas_recurrent_scan__compressed_kv_cla__dense_activation_gelu__decode_kernel(
    A_x: jax.Array,
    A_c_kv: jax.Array,
    A_w_q: jax.Array,
    A_w_uk: jax.Array,
    A_w_uv: jax.Array,
    A_w_o: jax.Array,
    B_x: jax.Array,
    B_w1: jax.Array,
    B_b1: jax.Array,
    B_w2: jax.Array,
    B_b2: jax.Array,
):
    return _impl(A_x, A_c_kv, A_w_q, A_w_uk, A_w_uv, A_w_o, B_x, B_w1, B_b1, B_w2, B_b2)
```

```python
import jax
import jax.numpy as jnp
from jax import lax
import jax.experimental.pallas as pl
import jax.experimental.pallas.tpu as pltpu

F32 = jnp.float32
BF16 = jnp.bfloat16
B, H, SK, D, M, DC, F = 2, 32, 16384, 128, 512, 512, 1792
LOG2E = 1.4426950408889634
NT = (((1,), (1,)), ((), ()))


def make_kernel(lead=26, ex=2, vpu=(128, 64, 32, 32), tiny=8, QU=4, IU=4, NM=5, NT0=6, vs=0, first=10, cs=5, ffn=0, flags=None, nocomp=False, wmode=0, prof=False):
    def mark(name):
        if prof:
            with jax.named_scope(name):
                pl.delay(1)

    NS = 8
    NCB = 32
    assert sum(vpu) == (8 - NT0) * D
    NV = NT0 - NM

    def kernel(x_hbm, ckv_hbm, wq_hbm, wuk_hbm, wuv_hbm, wo_hbm, w1_hbm, b1_hbm, w2_hbm, b2_hbm,
               o_ref,
               x_buf, b1_buf, b2_buf, c_buf, wq_buf, wuk_buf, wuv_buf, wo_buf, w1_buf, w2_buf,
               xb_ref, t8, qa_ref, acc_ref, m_ref, l_ref, a_buf, ctx_ref, cb_ref, sems, tsems, sem_small):
        def copy(src, dst, sem):
            return pltpu.make_async_copy(src, dst, sem)

        def wait_all(buf, sem):
            copy(buf, buf, sem).wait()

        def aligned(o, n):
            return pl.ds(o if isinstance(o, int) else pl.multiple_of(o, n), n)

        def weight(hbm, buf, sem):
            return lambda g, j: copy(hbm.at[16 * j + g], buf.at[g, j], sem(g >> 2))

        def ckv(g, j):
            src = (g & 64) * 8 + (g & 1) * 256 + ((g & 63) >> 1) + 32 * j
            return copy(ckv_hbm.at[src], c_buf.at[g, j], sems.at[(g >> 2) & (NS - 1)])

        def w1_piece(i, s):
            r = aligned(8 * i, 8)
            return copy(w1_hbm.at[r], w1_buf.at[r], tsems.at[s])

        def ffn_a(g, j):
            t = j >> 1
            r, c = (t & 1) * 4 + (t & 2) + (g & 1), g >> 1
            if j % 2 == ffn:
                rows = aligned(32 * (7 * r + c), 32)
                return copy(w2_hbm.at[rows], w2_buf.at[rows], tsems.at[g >> 2])
            return w1_piece(8 * r + c, g >> 2)

        def ffn_b(g, j):
            return w1_piece(8 * ((j >> 1) + 4 * (j & 1)) + 7, 3)

        late = [(r, c, 7) for c in range(12, 16) for r in range(NM)]
        late += [(r, c, 8 + ((c - 12) >> (2 - vs))) for c in range(12, 16) for r in range(NM, NT0)]

        def wo_late(g, j):
            r, c, s = late[8 * g + j]
            return copy(wo_hbm.at[16 * r + c], wo_buf.at[c, r], tsems.at[s])

        ends = [sum(vpu[:i + 1]) for i in range(len(vpu))]

        def last(n):
            d = n * tiny
            r, c, o = NT0 + d // D, 12 + d % D // 32, pl.ds(d % 32, tiny)
            return copy(wo_hbm.at[16 * r + c, o], wo_buf.at[c, r, o], tsems.at[12 + sum(d >= e for e in ends)])

        segs = [(16, weight(wq_hbm, wq_buf, lambda y: sems.at[y])), (16, weight(wuk_hbm, wuk_buf, lambda y: sems.at[4 + y])),
                (128, ckv), (16, weight(wuv_hbm, wuv_buf, lambda y: sems.at[y])), (14, ffn_a), (1, ffn_b),
                (12, weight(wo_hbm, wo_buf, lambda y: tsems.at[4 + y]))] + [(1, lambda g, j, i=i: wo_late(i, j)) for i in range(NT0 // 2)]
        n_groups = sum(n for n, _ in segs)
        n_last = ends[-1] // tiny

        def find(g):
            o = 0
            for n, f in segs:
                if o <= g < o + n:
                    return o, o + n, f
                o += n
            return (0, 0, None) if g < 0 else (o, g + 1, None)

        def step(g, at):
            for t in range(4):
                dg, t0 = divmod(t - lead, 4)
                o, _, f = find(at + dg)
                if f:
                    f(g + (dg - o), 2 * t0).start(priority=0)
                o, _, f = find(at)
                if f:
                    f(g - o, 2 * t + 1).start(priority=1)
                elif 4 * (at - o) + t < n_last:
                    last(4 * (at - o) + t).start(priority=1)

        def issue(lo, hi):
            while lo < hi:
                e = min([hi] + [find(lo + d)[1] - d for d in (0, -lead // 4, (3 - lead) // 4)])
                if e - lo == 1:
                    step(lo, lo)
                else:
                    pl.loop(lo, e)(lambda g: step(g, lo))
                lo = e

        def top_up(blk):
            issue(4 * (blk + 3) + ex, 4 * (blk + 4) + ex)

        x_copy = copy(x_hbm, x_buf, sem_small.at[0])
        b1_copy = copy(b1_hbm, b1_buf, sem_small.at[1])
        b2_copy = copy(b2_hbm, b2_buf, sem_small.at[1])
        issue(0, 1)
        x_copy.start()
        b1_copy.start()
        b2_copy.start()
        issue(1, first)

        x_copy.wait()
        x = x_buf[...].astype(F32)
        xc = x - jnp.mean(x, axis=-1, keepdims=True)
        var = jnp.mean(xc * xc, axis=-1, keepdims=True)
        xn = (xc * lax.rsqrt(var + 1e-5)).astype(BF16)
        xp = jnp.concatenate([xn.astype(F32), jnp.zeros((128 - B, M), F32)], axis=0)
        for j in range(M // 128):
            xt = xp[:, j * 128:(j + 1) * 128].T
            for b in range(B):
                xb_ref[b, j * 128:(j + 1) * 128, :] = jnp.broadcast_to(xt[:, b:b + 1], (128, 128))
        issue(first, 12 + ex)

        def q_slot(y, carry):
            mark('q_ready')
            wait_all(wq_buf.at[pl.ds(4 * y, 4)], sems.at[y])
            mark('q_arr')
            for t in range(4):
                pl.when(y == t)(lambda t=t: top_up(t))

            def q_body(t, carry):
                q0, q1 = carry
                for v in range(8):
                    r, c, e = t >> 1, (t & 1) * 2 + v // 4, v % 4
                    m = (16 * r + 4 * y + c) * 4 + e
                    w = wq_buf[4 * y + c, r, e].astype(F32)
                    q0 = q0 + xb_ref[0, pl.ds(m, 1), :] * w
                    q1 = q1 + xb_ref[1, pl.ds(m, 1), :] * w
                return q0, q1

            return lax.fori_loop(0, 16, q_body, carry)

        q01 = lax.fori_loop(0, 4, q_slot, (jnp.zeros((H, D), F32), jnp.zeros((H, D), F32)))
        q = jnp.concatenate([q01[0], q01[1], jnp.zeros((128 - B * H, D), F32)], axis=0).astype(BF16)

        group = (lax.broadcasted_iota(jnp.int32, (16, 8, 128), 2) % H) // 8

        @pl.loop(0, 4)
        def _(y):
            mark('k_ready')
            wait_all(wuk_buf.at[pl.ds(4 * y, 4)], sems.at[y + 4])
            mark('k_arr')
            for t in range(4):
                pl.when(y == t)(lambda t=t: top_up(4 + t))

            @pl.loop(0, 8, unroll=QU)
            def _(r):
                w = wuk_buf[pl.ds(4 * y, 4), r].reshape(16 * H, D)
                v = lax.dot_general(w, q, NT, preferred_element_type=F32).reshape(16, 4, 8, 128)
                v = jnp.where(group == 0, v[:, 0],
                              jnp.where(group == 1, v[:, 1], jnp.where(group == 2, v[:, 2], v[:, 3])))
                t8[aligned((4 * r + y) * 128, 128), :] = v.reshape(128, 128)

        sub = lax.broadcasted_iota(jnp.int32, (128, 128), 1) % 8

        @pl.loop(0, DC // 128)
        def _(j):
            t = t8[pl.ds(j * 1024, 128, stride=8), :]
            for s in range(1, 8):
                t = jnp.where(sub == s, t8[pl.ds(j * 1024 + s, 128, stride=8), :], t)
            qa_ref[j] = (t.T[:B * H] * (D ** -0.5 * LOG2E)).astype(BF16)

        m_ref[...] = jnp.full((B * H, 128), -jnp.inf, F32)
        l_ref[...] = jnp.zeros((B * H, 128), F32)
        acc_ref[...] = jnp.zeros((B * H, DC), F32)

        @pl.loop(0, NCB)
        def _(i):
            mark('c_ready')
            wait_all(c_buf.at[pl.ds(4 * i, 4)], sems.at[i & (NS - 1)])
            mark('c_arr')
            inner = NCB - 3 - (ex + 3) // 4
            pl.when(i < inner)(lambda: pl.loop(4 * (i + 11) + ex, 4 * (i + 12) + ex)(lambda g: step(g, 44)))
            for t in range(inner, NCB):
                pl.when(i == t)(lambda t=t: top_up(8 + t))
            hrows = aligned((i >> 4) * H, H)
            c = c_buf[pl.ds(4 * i, 4)].reshape(1024, DC)
            qa = jnp.concatenate([qa_ref[j, hrows, :] for j in range(DC // 128)], axis=1)
            sc = lax.dot_general(qa, c, NT, preferred_element_type=F32)
            m_prev = m_ref[hrows, :]
            m_new = jnp.maximum(m_prev, jnp.max(sc, axis=1, keepdims=True))
            p = jnp.exp2(sc - m_new[:, :1])
            alpha = jnp.exp2(m_prev - m_new)
            l_ref[hrows, :] = alpha * l_ref[hrows, :] + jnp.sum(p, axis=1, keepdims=True)
            m_ref[hrows, :] = m_new
            pv = jnp.dot(p.astype(BF16), c, preferred_element_type=F32)
            acc_ref[hrows, :] = acc_ref[hrows, :] * alpha[:, :1] + pv

        pc = (acc_ref[...] / l_ref[...][:, :1]).astype(BF16)
        pcs = jnp.concatenate([pc[:, j * 128:(j + 1) * 128] for j in range(DC // 128)], axis=0)
        lane = lax.broadcasted_iota(jnp.int32, (4 * B * H, 128), 1)
        diag = (lane % H) == lax.broadcasted_iota(jnp.int32, (4 * B * H, 128), 0) % H
        src = lax.broadcasted_iota(jnp.int32, (128, 128), 0) - lax.broadcasted_iota(jnp.int32, (128, 128), 1) // H

        def v_slot(y, ctx):
            @pl.loop(0, 2)
            def _(u):
                for c in range(4):
                    rep = jnp.dot(pcs, jnp.where(src == 4 * (16 * u + 4 * y + c), 1.0, 0.0).astype(BF16), preferred_element_type=F32)
                    a_buf[c, :, u] = jnp.where(diag, rep, 0.0).astype(BF16).reshape(4, B * H, 128)

            mark('v_ready')
            wait_all(wuv_buf.at[pl.ds(4 * y, 4)], sems.at[y])
            mark('v_arr')
            for t in range(4):
                pl.when(y == t)(lambda t=t: top_up(40 + t))
            lhs = jnp.concatenate([a_buf[c, i, u] for c in range(4) for i in range(4) for u in range(2)], axis=1)
            return ctx + jnp.dot(lhs, wuv_buf[pl.ds(4 * y, 4)].reshape(128 * H, D), preferred_element_type=F32)

        ctx_ref[:B * H] = lax.fori_loop(0, 4, v_slot, jnp.zeros((B * H, D), F32))

        def ctx_heads(y, n):
            v = jnp.concatenate([ctx_ref[pl.ds(4 * r + y, B, stride=H), :] for r in range(n)], axis=1)
            return jnp.concatenate([v, jnp.zeros((8 - B, n * D), F32)], axis=0).astype(BF16)

        @pl.loop(0, 8 - NM)
        def _(t):
            ct = jnp.concatenate([ctx_ref[pl.ds(4 * (NM + t) + 3, B, stride=H), :], jnp.zeros((128 - B, D), F32)], axis=0).T
            for b in range(B):
                cb_ref[b, aligned(t * D, D), :] = jnp.broadcast_to(ct[:, b:b + 1], (D, 128))

        b1_copy.wait()
        b2_copy.wait()
        for s in range(4):
            mark('f_ready')
            for g in range(4 * s, min(4 * s + 4, 15)):
                for j in range(8):
                    (ffn_a(g, j) if g < 14 else ffn_b(0, j)).wait()
            mark('f_arr')
            issue(4 * (47 + s) + ex, 4 * (47 + s) + ex + (4 if s < 3 else 3))
        done = 4 * 50 + ex + 3
        end = n_groups + (max(lead, n_last) + 3) // 4
        xn8 = jnp.concatenate([xn.astype(F32), jnp.zeros((8 - B, M), F32)], axis=0).astype(BF16)
        h = jnp.dot(xn8, w1_buf[...], preferred_element_type=F32) + b1_buf[...].astype(F32).reshape(1, F)
        h = jax.nn.gelu(h, approximate=True).astype(BF16)
        gg = jnp.dot(h, w2_buf[...], preferred_element_type=F32) + b2_buf[...].astype(F32).reshape(1, M)
        gate = gg * jax.nn.sigmoid(gg)

        def wo_heads(y, n):
            return jnp.concatenate([wo_buf[pl.ds(4 * y, 4), r].reshape(D, M) for r in range(n)], axis=0)

        def o_slot(y, s):
            lhs = ctx_heads(y, 8)
            mark('o_ready')
            wait_all(wo_buf.at[pl.ds(4 * y, 4)], tsems.at[4 + y])
            mark('o_arr')
            for t in range(3):
                pl.when(y == t)(lambda t=t: issue(done + 4 * t, done + 4 * t + 4 if t < 2 else end))
            return s + jnp.dot(lhs, wo_heads(y, 8), preferred_element_type=F32)

        s = lax.fori_loop(0, 3, o_slot, jnp.zeros((8, M), F32))
        lhs = ctx_heads(3, NM)
        mark('o_ready')
        wait_all(wo_buf.at[pl.ds(12, 4), pl.ds(0, NM)], tsems.at[7])
        mark('o_arr')
        s = s + jnp.dot(lhs, wo_heads(3, NM), preferred_element_type=F32)
        base = jnp.concatenate([x, jnp.zeros((8 - B, M), F32)], axis=0) + s * gate
        acc = [None] * B

        def vpu_rows(r, d):
            w = wo_buf[12 + d // 32, r, pl.ds(d % 32, 8), :].astype(F32)
            for b in range(B):
                t = w * jnp.concatenate([cb_ref[b, pl.ds((r - NM) * D + d, 8), :]] * (M // 128), axis=1)
                acc[b] = t if acc[b] is None else acc[b] + t

        for k in range(1 << vs if NV else 0):
            mark('t_ready')
            wait_all(wo_buf.at[pl.ds(12 + k * (4 >> vs), 4 >> vs), pl.ds(NM, NV)], tsems.at[8 + k])
            mark('t_arr')
            for r in range(NM, NT0):
                for d in range(k * (D >> vs), (k + 1) * (D >> vs), 8):
                    vpu_rows(r, d)
        o = 0
        for i, n in enumerate(vpu):
            mark('t_ready')
            for k in range(o // tiny, (o + n) // tiny):
                last(k).wait()
            mark('t_arr')
            for r0 in range(o, o + n, 8):
                vpu_rows(NT0 + r0 // D, r0 % D)
            o += n
        row = lax.broadcasted_iota(jnp.int32, (8, M), 0)
        r = [jnp.sum(acc[b], axis=0, keepdims=True) for b in range(B)]
        o_ref[...] = (base + jnp.where(row == 0, r[0], r[1]) * gate).astype(BF16)[:B]

    def fn(A_x, A_c_kv, A_w_q, A_w_uk, A_w_uv, A_w_o, B_x, B_w1, B_b1, B_w2, B_b2):
        del B_x
        W = (128, 4, H, D)
        WB = (16, 8, 4, H, D)
        out = pl.pallas_call(
            kernel,
            out_shape=jax.ShapeDtypeStruct((B, M), BF16),
            in_specs=[pl.BlockSpec(memory_space=pltpu.HBM)] * 10,
            out_specs=pl.BlockSpec(memory_space=pltpu.VMEM),
            scratch_shapes=[
                pltpu.VMEM((B, M), BF16), pltpu.VMEM((F,), BF16), pltpu.VMEM((M,), BF16),
                pltpu.VMEM((128, 8, 32, DC), BF16),
                pltpu.VMEM(WB, BF16), pltpu.VMEM(WB, BF16), pltpu.VMEM(WB, BF16),
                pltpu.VMEM((16, 8, 32, M), BF16), pltpu.VMEM((M, F), BF16), pltpu.VMEM((F, M), BF16),
                pltpu.VMEM((B, M, 128), F32),
                pltpu.VMEM((DC * 8 + 8, 128), F32),
                pltpu.VMEM((DC // 128, B * H, 128), BF16), pltpu.VMEM((B * H, DC), F32),
                pltpu.VMEM((B * H, 128), F32), pltpu.VMEM((B * H, 128), F32),
                pltpu.VMEM((4, 4, 2, B * H, 128), BF16), pltpu.VMEM(((B + 1) * H, D), F32),
                pltpu.VMEM((B, (8 - NM) * D, 128), F32),
                pltpu.SemaphoreType.DMA((NS,)), pltpu.SemaphoreType.DMA((12 + len(vpu),)), pltpu.SemaphoreType.DMA((2,)),
            ],
            compiler_params=pltpu.CompilerParams(vmem_limit_bytes=100 * 1024 * 1024, disable_bounds_checks=True,
                                                 disable_semaphore_checks=True, flags=flags),
        )(A_x.reshape(B, M), A_c_kv.reshape(B * SK // 32, 32, DC), A_w_q.reshape(W), A_w_uk.reshape(W), A_w_uv.reshape(W),
          A_w_o.reshape(H * D // 32, 32, M), B_w1, B_b1, B_w2, B_b2)
        return out.reshape(B, 1, M)
    return fn


_impl = make_kernel(**dict(first=12))


@jax.jit
def pallas_recurrent_scan__compressed_kv_cla__dense_activation_gelu__decode_kernel(
    A_x: jax.Array,
    A_c_kv: jax.Array,
    A_w_q: jax.Array,
    A_w_uk: jax.Array,
    A_w_uv: jax.Array,
    A_w_o: jax.Array,
    B_x: jax.Array,
    B_w1: jax.Array,
    B_b1: jax.Array,
    B_w2: jax.Array,
    B_b2: jax.Array,
):
    return _impl(A_x, A_c_kv, A_w_q, A_w_uk, A_w_uv, A_w_o, B_x, B_w1, B_b1, B_w2, B_b2)
```

```python
import jax
import jax.numpy as jnp
from jax import lax
import jax.experimental.pallas as pl
import jax.experimental.pallas.tpu as pltpu

F32 = jnp.float32
BF16 = jnp.bfloat16

B, H, SK, D, M, DC, F = 2, 32, 16384, 128, 512, 512, 1792
LOG2E = 1.4426950408889634
NT = (((1,), (1,)), ((), ()))

LEAD = 26
AHEAD = 16
NSEM = 8
NCB = 32
R_MXU = 5
R_SMALL = 6
SMALL_ROWS = (96, 64, 48, 32, 16)


def _kernel(x_hbm, ckv_hbm, wq_hbm, wuk_hbm, wuv_hbm, wo_hbm, w1_hbm, b1_hbm, w2_hbm, b2_hbm,
            o_ref,
            x_buf, b1_buf, b2_buf, c_buf, wq_buf, wuk_buf, wuv_buf, wo_buf, w1_buf, w2_buf,
            xb_ref, t8, qa_ref, acc_ref, m_ref, l_ref, a_buf, ctx_ref, cb_ref,
            sems, ffn_sems, wo_sems, small_sems, vec_sems):
    copy = pltpu.make_async_copy

    def wait_all(buf, sem):
        copy(buf, buf, sem).wait()

    def aligned(o, n):
        return pl.ds(o if isinstance(o, int) else pl.multiple_of(o, n), n)

    def block(y):
        return pl.ds(4 * y, 4)

    def pad_rows(v, n):
        return jnp.concatenate([v, jnp.zeros((n - v.shape[0], v.shape[1]), v.dtype)], axis=0)

    def weight(hbm, buf, sem, s0):
        return lambda g, j: copy(hbm.at[16 * j + g], buf.at[g, j], sem.at[s0 + (g >> 2)])

    def ckv(g, j):
        src = (g & 64) * 8 + (g & 1) * 256 + ((g & 63) >> 1) + 32 * j
        return copy(ckv_hbm.at[src], c_buf.at[g, j], sems.at[(g >> 2) & (NSEM - 1)])

    def w1_piece(i, s):
        rows = aligned(8 * i, 8)
        return copy(w1_hbm.at[rows], w1_buf.at[rows], ffn_sems.at[s])

    def ffn(g, j):
        t = j >> 1
        r, c = (t & 1) * 4 + (t & 2) + (g & 1), g >> 1
        if j % 2:
            return w1_piece(8 * r + c, g >> 2)
        rows = aligned(32 * (7 * r + c), 32)
        return copy(w2_hbm.at[rows], w2_buf.at[rows], ffn_sems.at[g >> 2])

    def ffn_rest(g, j):
        return w1_piece(8 * ((j >> 1) + 4 * (j & 1)) + 7, 3)

    late = [(r, c, 3) for c in range(12, 16) for r in range(R_MXU)]
    late += [(r, c, 4) for c in range(12, 16) for r in range(R_MXU, R_SMALL)]

    def wo_late(i):
        def member(g, j):
            r, c, s = late[8 * i + j]
            return copy(wo_hbm.at[16 * r + c], wo_buf.at[c, r], wo_sems.at[s])
        return member

    small_end = [sum(SMALL_ROWS[:i + 1]) for i in range(len(SMALL_ROWS))]

    def small(d):
        r, c, rows = R_SMALL + d // D, 12 + d % D // 32, pl.ds(d % 32, 8)
        sem = small_sems.at[sum(d >= e for e in small_end)]
        return copy(wo_hbm.at[16 * r + c, rows], wo_buf.at[c, r, rows], sem)

    segments = [(16, weight(wq_hbm, wq_buf, sems, 0)), (16, weight(wuk_hbm, wuk_buf, sems, 4)),
                (128, ckv), (16, weight(wuv_hbm, wuv_buf, sems, 0)),
                (14, ffn), (1, ffn_rest), (12, weight(wo_hbm, wo_buf, wo_sems, 0))]
    segments += [(1, wo_late(i)) for i in range(len(late) // 8)]
    n_groups = sum(n for n, _ in segments)
    n_small = small_end[-1] // 8
    n_steps = n_groups + (max(LEAD, n_small) + 3) // 4

    def find(g):
        o = 0
        for n, member in segments:
            if o <= g < o + n:
                return o, o + n, member
            o += n
        return (0, 0, None) if g < 0 else (o, g + 1, None)

    def step(g, at):
        for t in range(4):
            dg, t0 = divmod(t - LEAD, 4)
            o, _, member = find(at + dg)
            if member:
                member(g + (dg - o), 2 * t0).start(priority=0)
            o, _, member = find(at)
            if member:
                member(g - o, 2 * t + 1).start(priority=1)
            elif 4 * (at - o) + t < n_small:
                small(8 * (4 * (at - o) + t)).start(priority=1)

    def issue(lo, hi):
        while lo < hi:
            e = min([hi] + [find(lo + d)[1] - d for d in (0, -LEAD // 4, (3 - LEAD) // 4)])
            if e - lo == 1:
                step(lo, lo)
            else:
                pl.loop(lo, e)(lambda g: step(g, lo))
            lo = e

    def top_up(y, first, n):
        for t in range(n):
            o = 4 * (first + t) + AHEAD
            pl.when(y == t)(lambda o=o: issue(o, o + 4))

    x_copy = copy(x_hbm, x_buf, vec_sems.at[0])
    b1_copy = copy(b1_hbm, b1_buf, vec_sems.at[1])
    b2_copy = copy(b2_hbm, b2_buf, vec_sems.at[2])
    issue(0, 1)
    x_copy.start()
    b1_copy.start()
    b2_copy.start()
    issue(1, 12)

    x_copy.wait()
    x = x_buf[...].astype(F32)
    xc = x - jnp.mean(x, axis=-1, keepdims=True)
    var = jnp.mean(xc * xc, axis=-1, keepdims=True)
    xn = (xc * lax.rsqrt(var + 1e-5)).astype(BF16).astype(F32)
    xp = pad_rows(xn, 128)
    for j in range(M // 128):
        xt = xp[:, j * 128:(j + 1) * 128].T
        for b in range(B):
            xb_ref[b, j * 128:(j + 1) * 128, :] = jnp.broadcast_to(xt[:, b:b + 1], (128, 128))
    issue(12, AHEAD)

    def q_block(y, carry):
        wait_all(wq_buf.at[block(y)], sems.at[y])
        top_up(y, 0, 4)

        def body(t, carry):
            q0, q1 = carry
            for v in range(8):
                r, c, e = t >> 1, 4 * y + (t & 1) * 2 + v // 4, v % 4
                m = (16 * r + c) * 4 + e
                w = wq_buf[c, r, e].astype(F32)
                q0 = q0 + xb_ref[0, pl.ds(m, 1), :] * w
                q1 = q1 + xb_ref[1, pl.ds(m, 1), :] * w
            return q0, q1

        return lax.fori_loop(0, 16, body, carry)

    q = lax.fori_loop(0, 4, q_block, (jnp.zeros((H, D), F32), jnp.zeros((H, D), F32)))
    q = pad_rows(jnp.concatenate(q, axis=0), 128).astype(BF16)

    group = (lax.broadcasted_iota(jnp.int32, (16, 8, 128), 2) % H) // 8

    @pl.loop(0, 4)
    def _(y):
        wait_all(wuk_buf.at[block(y)], sems.at[4 + y])
        top_up(y, 4, 4)

        @pl.loop(0, 8, unroll=4)
        def _(r):
            w = wuk_buf[block(y), r].reshape(16 * H, D)
            v = lax.dot_general(w, q, NT, preferred_element_type=F32).reshape(16, 4, 8, 128)
            v = jnp.where(group == 0, v[:, 0],
                          jnp.where(group == 1, v[:, 1], jnp.where(group == 2, v[:, 2], v[:, 3])))
            t8[aligned((4 * r + y) * 128, 128), :] = v.reshape(128, 128)

    sub = lax.broadcasted_iota(jnp.int32, (128, 128), 1) % 8

    @pl.loop(0, DC // 128)
    def _(j):
        t = t8[pl.ds(j * 1024, 128, stride=8), :]
        for s in range(1, 8):
            t = jnp.where(sub == s, t8[pl.ds(j * 1024 + s, 128, stride=8), :], t)
        qa_ref[j] = (t.T[:B * H] * (D ** -0.5 * LOG2E)).astype(BF16)

    m_ref[...] = jnp.full((B * H, 128), -jnp.inf, F32)
    l_ref[...] = jnp.zeros((B * H, 128), F32)
    acc_ref[...] = jnp.zeros((B * H, DC), F32)
    inner = NCB - (AHEAD + 3) // 4

    @pl.loop(0, NCB)
    def _(i):
        wait_all(c_buf.at[block(i)], sems.at[i & (NSEM - 1)])

        @pl.when(i < inner)
        def _():
            o = 4 * (8 + i) + AHEAD
            pl.loop(o, o + 4)(lambda g: step(g, 32 + AHEAD))

        top_up(i - inner, 8 + inner, NCB - inner)
        hrows = aligned((i >> 4) * H, H)
        c = c_buf[block(i)].reshape(1024, DC)
        qa = jnp.concatenate([qa_ref[j, hrows, :] for j in range(DC // 128)], axis=1)
        sc = lax.dot_general(qa, c, NT, preferred_element_type=F32)
        m_prev = m_ref[hrows, :]
        m_new = jnp.maximum(m_prev, jnp.max(sc, axis=1, keepdims=True))
        p = jnp.exp2(sc - m_new[:, :1])
        alpha = jnp.exp2(m_prev - m_new)
        l_ref[hrows, :] = alpha * l_ref[hrows, :] + jnp.sum(p, axis=1, keepdims=True)
        m_ref[hrows, :] = m_new
        pv = jnp.dot(p.astype(BF16), c, preferred_element_type=F32)
        acc_ref[hrows, :] = acc_ref[hrows, :] * alpha[:, :1] + pv

    pc = (acc_ref[...] / l_ref[...][:, :1]).astype(BF16)
    pcs = jnp.concatenate([pc[:, j * 128:(j + 1) * 128] for j in range(DC // 128)], axis=0)
    diag = (lax.broadcasted_iota(jnp.int32, (4 * B * H, 128), 1) % H
            == lax.broadcasted_iota(jnp.int32, (4 * B * H, 128), 0) % H)
    shift = (lax.broadcasted_iota(jnp.int32, (128, 128), 0)
             - lax.broadcasted_iota(jnp.int32, (128, 128), 1) // H)

    def ctx_block(y, ctx):
        @pl.loop(0, 2)
        def _(u):
            for c in range(4):
                pick = jnp.where(shift == 4 * (16 * u + 4 * y + c), 1.0, 0.0).astype(BF16)
                rep = jnp.dot(pcs, pick, preferred_element_type=F32)
                a_buf[c, :, u] = jnp.where(diag, rep, 0.0).astype(BF16).reshape(4, B * H, 128)

        wait_all(wuv_buf.at[block(y)], sems.at[y])
        top_up(y, 40, 4)
        lhs = jnp.concatenate([a_buf[c, i, u] for c in range(4) for i in range(4) for u in range(2)], axis=1)
        return ctx + jnp.dot(lhs, wuv_buf[block(y)].reshape(128 * H, D), preferred_element_type=F32)

    ctx_ref[:B * H] = lax.fori_loop(0, 4, ctx_block, jnp.zeros((B * H, D), F32))

    def ctx_head(h):
        return ctx_ref[pl.ds(h, B, stride=H), :]

    @pl.loop(0, 8 - R_MXU)
    def _(t):
        ct = pad_rows(ctx_head(4 * (R_MXU + t) + 3), 128).T
        for b in range(B):
            cb_ref[b, aligned(t * D, D), :] = jnp.broadcast_to(ct[:, b:b + 1], (D, 128))

    b1_copy.wait()
    b2_copy.wait()
    done = 4 * 44 + AHEAD
    for s in range(4):
        groups = range(4 * s, min(4 * s + 4, 15))
        for g in groups:
            for j in range(8):
                (ffn if g < 14 else ffn_rest)(g, j).wait()
        issue(done, done + len(groups))
        done += len(groups)
    h = jnp.dot(pad_rows(xn, 8).astype(BF16), w1_buf[...], preferred_element_type=F32)
    h = jax.nn.gelu(h + b1_buf[...].astype(F32).reshape(1, F), approximate=True).astype(BF16)
    gg = jnp.dot(h, w2_buf[...], preferred_element_type=F32) + b2_buf[...].astype(F32).reshape(1, M)
    gate = gg * jax.nn.sigmoid(gg)

    def wo_lhs(y, n):
        return pad_rows(jnp.concatenate([ctx_head(4 * r + y) for r in range(n)], axis=1), 8).astype(BF16)

    def wo_dot(lhs, y, n):
        w = jnp.concatenate([wo_buf[block(y), r].reshape(D, M) for r in range(n)], axis=0)
        return jnp.dot(lhs, w, preferred_element_type=F32)

    def wo_block(y, s):
        lhs = wo_lhs(y, 8)
        wait_all(wo_buf.at[block(y)], wo_sems.at[y])
        for t in range(3):
            pl.when(y == t)(lambda t=t: issue(done + 4 * t, done + 4 * t + 4 if t < 2 else n_steps))
        return s + wo_dot(lhs, y, 8)

    s = lax.fori_loop(0, 3, wo_block, jnp.zeros((8, M), F32))
    lhs = wo_lhs(3, R_MXU)
    wait_all(wo_buf.at[block(3), pl.ds(0, R_MXU)], wo_sems.at[3])
    base = pad_rows(x, 8) + (s + wo_dot(lhs, 3, R_MXU)) * gate
    acc = [None] * B

    def vpu_rows(r, d):
        w = wo_buf[12 + d // 32, r, pl.ds(d % 32, 8), :].astype(F32)
        for b in range(B):
            a = cb_ref[b, pl.ds((r - R_MXU) * D + d, 8), :]
            t = w * jnp.concatenate([a] * (M // 128), axis=1)
            acc[b] = t if acc[b] is None else acc[b] + t

    wait_all(wo_buf.at[block(3), pl.ds(R_MXU, R_SMALL - R_MXU)], wo_sems.at[4])
    for r in range(R_MXU, R_SMALL):
        for d in range(0, D, 8):
            vpu_rows(r, d)
    for lo, hi in zip([0] + small_end, small_end):
        for d in range(lo, hi, 8):
            small(d).wait()
        for d in range(lo, hi, 8):
            vpu_rows(R_SMALL + d // D, d % D)
    rest = [jnp.sum(acc[b], axis=0, keepdims=True) for b in range(B)]
    rest = jnp.where(lax.broadcasted_iota(jnp.int32, (8, M), 0) == 0, rest[0], rest[1])
    o_ref[...] = (base + rest * gate).astype(BF16)[:B]


@jax.jit
def pallas_recurrent_scan__compressed_kv_cla__dense_activation_gelu__decode_kernel(
    A_x: jax.Array,
    A_c_kv: jax.Array,
    A_w_q: jax.Array,
    A_w_uk: jax.Array,
    A_w_uv: jax.Array,
    A_w_o: jax.Array,
    B_x: jax.Array,
    B_w1: jax.Array,
    B_b1: jax.Array,
    B_w2: jax.Array,
    B_b2: jax.Array,
):
    del B_x
    w_granules = (128, 4, H, D)
    w_groups = (16, 8, 4, H, D)
    dma = pltpu.SemaphoreType.DMA
    out = pl.pallas_call(
        _kernel,
        out_shape=jax.ShapeDtypeStruct((B, M), BF16),
        in_specs=[pl.BlockSpec(memory_space=pltpu.HBM)] * 10,
        out_specs=pl.BlockSpec(memory_space=pltpu.VMEM),
        scratch_shapes=[
            pltpu.VMEM((B, M), BF16), pltpu.VMEM((F,), BF16), pltpu.VMEM((M,), BF16),
            pltpu.VMEM((4 * NCB, 8, 32, DC), BF16),
            pltpu.VMEM(w_groups, BF16), pltpu.VMEM(w_groups, BF16), pltpu.VMEM(w_groups, BF16),
            pltpu.VMEM((16, 8, 32, M), BF16), pltpu.VMEM((M, F), BF16), pltpu.VMEM((F, M), BF16),
            pltpu.VMEM((B, M, 128), F32),
            pltpu.VMEM((DC * 8 + 8, 128), F32),
            pltpu.VMEM((DC // 128, B * H, 128), BF16), pltpu.VMEM((B * H, DC), F32),
            pltpu.VMEM((B * H, 128), F32), pltpu.VMEM((B * H, 128), F32),
            pltpu.VMEM((4, 4, 2, B * H, 128), BF16), pltpu.VMEM(((B + 1) * H, D), F32),
            pltpu.VMEM((B, (8 - R_MXU) * D, 128), F32),
            dma((NSEM,)), dma((4,)), dma((5,)), dma((len(SMALL_ROWS),)), dma((3,)),
        ],
        compiler_params=pltpu.CompilerParams(
            vmem_limit_bytes=100 * 1024 * 1024, disable_bounds_checks=True, disable_semaphore_checks=True),
    )(A_x.reshape(B, M), A_c_kv.reshape(B * SK // 32, 32, DC), A_w_q.reshape(w_granules),
      A_w_uk.reshape(w_granules), A_w_uv.reshape(w_granules), A_w_o.reshape(H * D // 32, 32, M),
      B_w1, B_b1, B_w2, B_b2)
    return out.reshape(B, 1, M)
```
